```python
import jax
import jax.numpy as jnp

def _softmax(x, axis=-1):
    return jax.nn.softmax(x, axis=axis)
def _gelu(x):
    return jax.nn.gelu(x, approximate=True)
def _silu(x):
    return jax.nn.silu(x)
def _sigmoid(x):
    return jax.nn.sigmoid(x)
def _layernorm(x, axis=-1, eps=1e-5):
    m = jnp.mean(x, axis=axis, keepdims=True)
    v = jnp.var(x, axis=axis, keepdims=True)
    return (x - m) / jnp.sqrt(v + eps)
def _scatter_add(tgt, idx, src, axis=0):
    return tgt.at[idx].add(src)
def _segment_sum(src, seg, n):
    return jax.ops.segment_sum(src, seg, n)
class _Rng:
    def __init__(self, key):
        self._k = key
    def _next(self):
        self._k, sub = jax.random.split(self._k)
        return sub
    def normal(self, shape):
        return jax.random.normal(self._next(), shape, dtype=jnp.bfloat16)
    def randint(self, lo, hi, shape):
        return jax.random.randint(self._next(), shape, lo, hi, dtype=jnp.int32)
    def uniform(self, shape, lo=0.0, hi=1.0):
        return jax.random.uniform(self._next(), shape, jnp.bfloat16, lo, hi)
    def permutation(self, n):
        return jax.random.permutation(self._next(), n)


kernel_name = 'concat_heads__gqa_block_cached__compressed_kv_cla__decode'

def setup_inputs():
    _rng = _Rng(jax.random.key(int.from_bytes(__import__("os").urandom(4), "little")))
    _w = (lambda a: (lambda t: t.astype(jnp.bfloat16) if jnp.issubdtype(t.dtype, jnp.floating) else t)(jnp.asarray(a)))
    def _A_setup():
        B, Sq, D = 2, 1, 512
        Hq, Hkv, Sk, Dh = 32, 32, 8192, 128
        assert Hq % Hkv == 0, (Hq, Hkv)
        return {
            "x": _w((lambda *s: _rng.normal(s) * 0.05)(B, Sq, D)),
            "k_cache": _w((lambda *s: _rng.normal(s) * 0.05)(B, Hkv, Sk, Dh)),
            "v_cache": _w((lambda *s: _rng.normal(s) * 0.05)(B, Hkv, Sk, Dh)),
            "wq": _w((lambda *s: _rng.normal(s) * 0.05)(D, Hq * Dh) * (D ** -0.5)),
            "wo": _w((lambda *s: _rng.normal(s) * 0.05)(Hq * Dh, D) * ((Hq * Dh) ** -0.5)),
        }
    _A_in = _A_setup()

    def _B_setup():
        B, H, Sq, Sk, D, M = 2, 32, 1, 8192, 128, 512
        Dc = 4 * D
        return {
            "x": _w((lambda *s: _rng.normal(s) * 0.05)(B, Sq, M)),
            "c_kv": _w((lambda *s: _rng.normal(s) * 0.05)(B, Sk, Dc)),
            "w_q": _w((lambda *s: _rng.normal(s) * 0.05)(M, H, D) * (M ** -0.5)),
            "w_uk": _w((lambda *s: _rng.normal(s) * 0.05)(Dc, H, D) * (Dc ** -0.5)),
            "w_uv": _w((lambda *s: _rng.normal(s) * 0.05)(Dc, H, D) * (Dc ** -0.5)),
            "w_o": _w((lambda *s: _rng.normal(s) * 0.05)(H, D, M) * ((H * D) ** -0.5)),
        }
    _B_in = _B_setup()

    return {
        "A_x": _A_in["x"],
        "A_k_cache": _A_in["k_cache"],
        "A_v_cache": _A_in["v_cache"],
        "A_wq": _A_in["wq"],
        "A_wo": _A_in["wo"],
        "B_x": _B_in["x"],
        "B_c_kv": _B_in["c_kv"],
        "B_w_q": _B_in["w_q"],
        "B_w_uk": _B_in["w_uk"],
        "B_w_uv": _B_in["w_uv"],
        "B_w_o": _B_in["w_o"],
    }

def reference(A_x, A_k_cache, A_v_cache, A_wq, A_wo, B_x, B_c_kv, B_w_q, B_w_uk, B_w_uv, B_w_o):
    def _A_ref(x, k_cache, v_cache, wq, wo):
        B, Sq, D = x.shape
        Hq, Dh = 32, 128
        Hkv = k_cache.shape[1]
        rep = Hq // Hkv
        q = (lambda x, *d: x.transpose(*d))((x @ wq).reshape(B, Sq, Hq, Dh), 0, 2, 1, 3)
        k = jnp.repeat(k_cache, rep, axis=1)
        v = jnp.repeat(v_cache, rep, axis=1)
        scores = jnp.einsum("bhqd,bhkd->bhqk", q, k) * (Dh ** -0.5)
        p = _softmax(scores, axis=-1)
        o = jnp.einsum("bhqk,bhkd->bhqd", p, v)
        return (lambda x, *d: x.transpose(*d))(o, 0, 2, 1, 3).reshape(B, Sq, Hq * Dh) @ wo

    def _B_ref(x, c_kv, w_q, w_uk, w_uv, w_o):
        B, Sq, M = x.shape[0], x.shape[1], x.shape[2]
        Sk = c_kv.shape[1]
        H, D = w_q.shape[1], w_q.shape[2]
        q = jnp.einsum("bqm,mhd->bhqd", x, w_q)
        k = jnp.einsum("bkc,chd->bhkd", c_kv, w_uk)
        v = jnp.einsum("bkc,chd->bhkd", c_kv, w_uv)
        scores = jnp.einsum("bhqd,bhkd->bhqk", q, k) * (D ** -0.5)
        off = Sk - Sq
        qi = jnp.arange(Sq)[:, None]
        kj = jnp.arange(Sk)[None, :]
        cmask = kj <= (qi + off)
        scores = jnp.where(cmask[None, None], scores, -1e9)
        p = _softmax(scores, axis=-1)
        ctx = jnp.einsum("bhqk,bhkd->bhqd", p, v)
        return jnp.einsum("bhqd,hdm->bqm", ctx, w_o)

    a = _A_ref(A_x, A_k_cache, A_v_cache, A_wq, A_wo)
    b = _B_ref(B_x, B_c_kv, B_w_q, B_w_uk, B_w_uv, B_w_o)
    return jnp.concatenate([a, b], axis=-1)
```

```python
import functools

import jax
import jax.numpy as jnp
from jax import lax
import jax.experimental.pallas as pl
import jax.experimental.pallas.tpu as pltpu

_NT = (((1,), (1,)), ((), ()))
_BF16 = jnp.bfloat16
_F32 = jnp.float32


def _dot(a, b):
    return jnp.dot(a, b, preferred_element_type=_F32)


def _dot_nt(a, b):
    return lax.dot_general(a, b, _NT, preferred_element_type=_F32)


def _build(B, H, S, D, M, C=128, P=4, XK=8, BV=12, CB=1024):
    R = C * P
    G = S // R
    NBH = B * H
    NP = NBH * G
    NK = XK + 2
    NV = BV + 2
    scale = float(D) ** -0.5
    HD = H * D

    def kernel(xa_hbm, k_hbm, v_hbm, wq_hbm, wo_hbm, xb_hbm, ckv_hbm, wqb_hbm,
               wuk_hbm, wuv_hbm, wob_hbm, out_ref,
               xa_buf, xb_buf, wq_buf, wo_buf, wqb_buf, wuk_buf, wuv_buf, wob_buf,
               ckv_buf, kbuf, vbuf, q_scr, s_scr, p_scr, l_scr, acc_scr, oa_scr,
               qabs_scr, sb_scr, ctxl_scr, ctxc_scr, semw, semk, semv):
        def bulk(src, dst, idx):
            return pltpu.make_async_copy(src, dst, semw.at[idx])

        cp_xa = bulk(xa_hbm, xa_buf, 0)
        cp_xb = bulk(xb_hbm, xb_buf, 1)
        cp_wq = bulk(wq_hbm, wq_buf, 2)
        cp_wqb = bulk(wqb_hbm, wqb_buf, 3)
        cp_wuk = bulk(wuk_hbm, wuk_buf, 4)
        cp_ckv = [bulk(ckv_hbm.at[b], ckv_buf.at[b], 5 + b) for b in range(B)]
        cp_wuv = bulk(wuv_hbm, wuv_buf, 5 + B)
        cp_wob = bulk(wob_hbm, wob_buf, 6 + B)
        cp_wo = bulk(wo_hbm, wo_buf, 7 + B)

        def kcp(i, c):
            slot = i % NK
            return pltpu.make_async_copy(
                k_hbm.at[pl.ds(i * R + c * C, C)],
                kbuf.at[slot, pl.ds(c * C, C)], semk.at[slot])

        def vcp(i, c):
            slot = i % NV
            return pltpu.make_async_copy(
                v_hbm.at[pl.ds(i * R + c * C, C)],
                vbuf.at[slot, pl.ds(c * C, C)], semv.at[slot])

        def kwait_all(i):
            slot = i % NK
            pltpu.make_async_copy(kbuf.at[slot], kbuf.at[slot], semk.at[slot]).wait()

        cp_xa.start()
        cp_xb.start()
        cp_wq.start()
        for i in range(XK):
            for c in range(P):
                kcp(i, c).start(priority=0)
        for cp in [cp_wqb, cp_wuk] + cp_ckv + [cp_wuv, cp_wob, cp_wo]:
            cp.start(priority=1)
        for i in range(BV):
            for c in range(P):
                vcp(i, c).start(priority=1)

        def rows8(r0, r1):
            n = r0.shape[-1]
            row = lax.broadcasted_iota(jnp.int32, (8, n), 0)
            z = jnp.where(row == 0, jnp.broadcast_to(r0, (8, n)),
                          jnp.where(row == 1, jnp.broadcast_to(r1, (8, n)), 0.0))
            return z.astype(_BF16)

        def head_pair(w_buf, hp):
            w = w_buf.bitcast(jnp.uint32)[pl.ds(hp, M, stride=H // 2), :]
            even = pltpu.bitcast(w << 16, _F32).astype(_BF16)
            odd = pltpu.bitcast(w & jnp.uint32(0xFFFF0000), _F32).astype(_BF16)
            return even, odd

        def qk(i):
            n = i // G
            j = i % G
            q = q_scr[n % H]
            s_scr[:, pl.ds(pl.multiple_of(j * R, R), R)] = _dot_nt(q, kbuf[i % NK])

        def softmax(n):
            s = s_scr[...]
            m = jnp.max(s, axis=1, keepdims=True)
            p = jnp.exp((s - m) * scale)
            l_scr[n % 2] = jnp.broadcast_to(jnp.sum(p, axis=1, keepdims=True), (8, D))
            p_scr[n % 2] = p.astype(_BF16)

        def pv(i):
            n = i // G
            j = i % G
            p = p_scr[n % 2, :, pl.ds(pl.multiple_of(j * R, R), R)]
            acc_scr[...] += _dot(p, vbuf[i % NV])

        cp_xa.wait()
        cp_wq.wait()
        xa8 = rows8(xa_buf[0].astype(_F32), xa_buf[1].astype(_F32))
        qa = _dot(xa8, wq_buf[...]).astype(_BF16)
        for h in range(H):
            q_scr[h] = qa[:, h * D:(h + 1) * D]

        acc_scr[...] = jnp.zeros_like(acc_scr)
        oa_scr[...] = jnp.zeros_like(oa_scr)

        def first_head(i, carry):
            kwait_all(i)
            for c in range(P):
                kcp(i + XK, c).start(priority=0)
            qk(i)
            return carry

        lax.fori_loop(0, G, first_head, 0)
        softmax(0)
        kwait_all(G)

        cp_xb.wait()
        cp_wqb.wait()
        cp_wuk.wait()
        xb8 = rows8(xb_buf[0].astype(_F32), xb_buf[1].astype(_F32))
        for hp in range(H // 2):
            wq_pair = head_pair(wqb_buf, hp)
            uk_pair = head_pair(wuk_buf, hp)
            for e in range(2):
                h = 2 * hp + e
                qh = _dot(xb8, wq_pair[e]).astype(_BF16)
                qabs = _dot_nt(qh, uk_pair[e])
                for b in range(B):
                    qabs_scr[b, h:h + 1, :] = qabs[b:b + 1, :]

        def fold(x, op):
            r = x[:, 0:128]
            for t in range(1, CB // 128):
                r = op(r, x[:, t * 128:(t + 1) * 128])
            return r

        for b in range(B):
            cp_ckv[b].wait()
            qab = qabs_scr[b].astype(_BF16)

            def b_scores(j, mx, b=b, qab=qab):
                off = pl.multiple_of(j * CB, CB)
                s = _dot_nt(qab, ckv_buf[b, pl.ds(off, CB), :])
                sb_scr[:, pl.ds(off, CB)] = s
                return jnp.maximum(mx, fold(s, jnp.maximum))

            mx = lax.fori_loop(0, S // CB, b_scores,
                               jnp.full((H, 128), -jnp.inf, _F32))
            m = jnp.max(mx, axis=1, keepdims=True)

            def b_ctx(j, carry, b=b, m=m):
                lsum, ctx = carry
                off = pl.multiple_of(j * CB, CB)
                p = jnp.exp((sb_scr[:, pl.ds(off, CB)] - m) * scale)
                ctx = ctx + _dot(p.astype(_BF16), ckv_buf[b, pl.ds(off, CB), :])
                return lsum + fold(p, jnp.add), ctx

            lsum, ctx = lax.fori_loop(
                0, S // CB, b_ctx,
                (jnp.zeros((H, 128), _F32), jnp.zeros((H, M), _F32)))
            ctxl_scr[b] = ctx / jnp.sum(lsum, axis=1, keepdims=True)

        cp_wuv.wait()
        for hp in range(H // 2):
            uv_pair = head_pair(wuv_buf, hp)
            for e in range(2):
                h = 2 * hp + e
                lhs = rows8(ctxl_scr[0, h:h + 1, :], ctxl_scr[1, h:h + 1, :])
                ctxc_scr[:, h * D:(h + 1) * D] = _dot(lhs, uv_pair[e])
        cp_wob.wait()
        ob = _dot(ctxc_scr[...].astype(_BF16), wob_buf[...])
        for b in range(B):
            out_ref[b, :, M:2 * M] = ob[b:b + 1, :].astype(out_ref.dtype)
        cp_wo.wait()

        def body(i, carry):
            def issue(c):
                @pl.when(i + G + XK < NP)
                def _():
                    kcp(i + G + XK, c).start(priority=0)

                @pl.when(i + BV < NP)
                def _():
                    vcp(i + BV, c).start(priority=1)

            vcp(i, 0).wait()
            issue(0)

            @pl.when(i + G < NP)
            def _():
                qk(i + G)

            for c in range(1, P):
                vcp(i, c).wait()
                issue(c)
            pv(i)

            @pl.when(i + G + 1 < NP)
            def _():
                kwait_all(i + G + 1)

            @pl.when(i % G == G - 1)
            def _():
                n = i // G
                o = (acc_scr[...] / l_scr[n % 2]).astype(_BF16)
                acc_scr[...] = jnp.zeros_like(acc_scr)
                h = n % H
                y = _dot(o, wo_buf[pl.ds(pl.multiple_of(h * D, D), D), :])
                row = lax.broadcasted_iota(jnp.int32, y.shape, 0)
                oa_scr[...] += jnp.where(row == n // H, y, 0.0)

                @pl.when(n + 1 < NBH)
                def _():
                    softmax(n + 1)

            return carry

        lax.fori_loop(0, NP, body, 0)
        oa = oa_scr[...]
        for b in range(B):
            out_ref[b, :, 0:M] = oa[b:b + 1, :].astype(out_ref.dtype)

    scratch = [
        pltpu.VMEM((B, 1, M), _BF16),
        pltpu.VMEM((B, 1, M), _BF16),
        pltpu.VMEM((M, HD), _BF16),
        pltpu.VMEM((HD, M), _BF16),
        pltpu.VMEM((M * H, D), _BF16),
        pltpu.VMEM((M * H, D), _BF16),
        pltpu.VMEM((M * H, D), _BF16),
        pltpu.VMEM((HD, M), _BF16),
        pltpu.VMEM((B, S, M), _BF16),
        pltpu.VMEM((NK, R, D), _BF16),
        pltpu.VMEM((NV, R, D), _BF16),
        pltpu.VMEM((H, 8, D), _BF16),
        pltpu.VMEM((8, S), _F32),
        pltpu.VMEM((2, 8, S), _BF16),
        pltpu.VMEM((2, 8, D), _F32),
        pltpu.VMEM((8, D), _F32),
        pltpu.VMEM((8, M), _F32),
        pltpu.VMEM((B, H, M), _F32),
        pltpu.VMEM((H, S), _F32),
        pltpu.VMEM((B, H, M), _F32),
        pltpu.VMEM((8, HD), _F32),
        pltpu.SemaphoreType.DMA((8 + B,)),
        pltpu.SemaphoreType.DMA((NK,)),
        pltpu.SemaphoreType.DMA((NV,)),
    ]

    def call(A_x, A_k_cache, A_v_cache, A_wq, A_wo, B_x, B_c_kv, B_w_q, B_w_uk,
             B_w_uv, B_w_o):
        any_spec = pl.BlockSpec(memory_space=pl.ANY)
        return pl.pallas_call(
            kernel,
            out_shape=jax.ShapeDtypeStruct((B, 1, 2 * M), _BF16),
            in_specs=[any_spec] * 11,
            out_specs=pl.BlockSpec(memory_space=pltpu.VMEM),
            scratch_shapes=scratch,
            compiler_params=pltpu.CompilerParams(
                vmem_limit_bytes=100 * 1024 * 1024),
        )(
            A_x,
            A_k_cache.reshape(NBH * S, D),
            A_v_cache.reshape(NBH * S, D),
            A_wq,
            A_wo,
            B_x,
            B_c_kv,
            B_w_q.reshape(M * H, D),
            B_w_uk.reshape(M * H, D),
            B_w_uv.reshape(M * H, D),
            B_w_o.reshape(HD, M),
        )

    return call


@jax.jit
def pallas_concat_heads__gqa_block_cached__compressed_kv_cla__decode_kernel(
    A_x: jax.Array,
    A_k_cache: jax.Array,
    A_v_cache: jax.Array,
    A_wq: jax.Array,
    A_wo: jax.Array,
    B_x: jax.Array,
    B_c_kv: jax.Array,
    B_w_q: jax.Array,
    B_w_uk: jax.Array,
    B_w_uv: jax.Array,
    B_w_o: jax.Array,
):
    B, H, S, D = A_k_cache.shape
    M = A_x.shape[-1]
    assert B == 2 and A_x.shape[1] == 1 and B_x.shape[1] == 1
    assert A_wq.shape == (M, H * D) and B_c_kv.shape == (B, S, M)
    assert B_w_q.shape == (M, H, D) and B_w_o.shape == (H, D, M)
    return _build(B, H, S, D, M)(A_x, A_k_cache, A_v_cache, A_wq, A_wo, B_x,
                                 B_c_kv, B_w_q, B_w_uk, B_w_uv, B_w_o)
```

```python
import functools

import jax
import jax.numpy as jnp
from jax import lax
import jax.experimental.pallas as pl
import jax.experimental.pallas.tpu as pltpu

_NT = (((1,), (1,)), ((), ()))
_BF16 = jnp.bfloat16
_F32 = jnp.float32
_HI, _LO = 0, 1


def _dot(a, b):
    return jnp.dot(a, b, preferred_element_type=_F32)


def _dot_nt(a, b):
    return lax.dot_general(a, b, _NT, preferred_element_type=_F32)


def _mult(x, m):
    return x if isinstance(x, int) else pl.multiple_of(x, m)


def _build(B, H, S, D, M, XK=6, BV=6, KB=1024, CB=256, tail_hi=True):
    R = 8
    C = 16
    KP = 128
    P = KP // C
    G = KB // KP
    PPG = S // KP
    NBH = B * H
    GPB = H // R
    NG = NBH // R
    NP = NG * PPG
    NK = XK + 2
    NV = BV + 2
    HD = H * D
    scale = float(D) ** -0.5
    UD = 128
    UI = UD // P
    assert XK == BV and BV < UI
    assert M == 512 and D == 128 and HD == 4096 and B == 2

    def kernel(xa_hbm, k_hbm, v_hbm, wq_hbm, wo_hbm, xb_hbm, ckv_hbm, wqb_hbm,
               wuk_hbm, wuv_hbm, wob_hbm, out_ref,
               xa_buf, xb_buf, wq_buf, wo_buf, wqb_buf, wuk_buf, wuv_buf, wob_buf,
               ckv_buf, kbuf, vbuf, q_scr, s_scr, p_scr, m_scr, l_scr, acc_scr,
               oa_scr, xb16_scr, qb_scr, qabs_scr, qab_scr, sb_scr, mb_scr, lb_scr, ctx_scr,
               ctxc_scr, ob_scr, semx, semu, semk, semv):
        cp_xa = pltpu.make_async_copy(xa_hbm, xa_buf, semx.at[0])
        cp_xb = pltpu.make_async_copy(xb_hbm, xb_buf, semx.at[1])

        def unit_wq(j):
            idx = (slice(None), pl.ds(_mult((j // 16) * 8, 8), 8),
                   pl.ds(_mult((j % 16) * 256, 256), 256))
            return wq_hbm.at[idx], wq_buf.at[idx]

        def unit_rows(hbm, buf):
            def f(j):
                idx = (slice(None), pl.ds(_mult(j * 32, 32), 32), slice(None))
                return hbm.at[idx], buf.at[idx]
            return f

        def unit_wide(hbm, buf, r0=0, row0=0):
            def f(j):
                idx = (pl.ds(r0, 4), pl.ds(_mult(row0 + j * 8, 8), 8), slice(None))
                return hbm.at[idx], buf.at[idx]
            return f

        segs = [
            (unit_wq, unit_rows(wqb_hbm, wqb_buf)),
            (unit_rows(wuk_hbm, wuk_buf), unit_wide(ckv_hbm, ckv_buf, 0, 0)),
            (unit_wide(ckv_hbm, ckv_buf, 0, 1024), unit_wide(ckv_hbm, ckv_buf, 4, 0)),
            (unit_wide(ckv_hbm, ckv_buf, 4, 1024), unit_rows(wuv_hbm, wuv_buf)),
            (unit_wide(wo_hbm, wo_buf), unit_wide(wob_hbm, wob_buf)),
        ]
        NSEG = len(segs)

        def ucp(seg, side, j):
            src, dst = segs[seg][side](j)
            return pltpu.make_async_copy(src, dst, semu.at[2 * seg + side])

        def uwait_all(seg):
            pltpu.make_async_copy(wo_buf, wo_buf, semu.at[2 * seg]).wait()

        def kv_src(hbm, i, c):
            g = i // PPG
            j = i % PPG
            return hbm.at[pl.ds(g * R, R), pl.ds(_mult(j * KP + c * C, C), C), :]

        def kcp(i, c):
            slot = i % NK
            return pltpu.make_async_copy(
                kv_src(k_hbm, i, c), kbuf.at[slot, :, pl.ds(c * C, C), :],
                semk.at[slot])

        def vcp(i, c):
            slot = i % NV
            return pltpu.make_async_copy(
                kv_src(v_hbm, i, c), vbuf.at[slot, :, pl.ds(c * C, C), :],
                semv.at[slot])

        def kwait_all(i):
            slot = i % NK
            pltpu.make_async_copy(kbuf.at[slot], kbuf.at[slot], semk.at[slot]).wait()

        def x16(buf):
            x = buf[...].astype(_F32)
            row = lax.broadcasted_iota(jnp.int32, (16, M), 0)
            z = jnp.where(row < 8, jnp.broadcast_to(x[0:1, :], (16, M)),
                          jnp.broadcast_to(x[1:2, :], (16, M)))
            return z.astype(_BF16)

        def pick(parts, k0=0):
            shape = parts[0].shape
            k = lax.broadcasted_iota(jnp.int32, shape, 0) % 8
            res = parts[0]
            for j in range(1, len(parts)):
                res = jnp.where(k == k0 + j, parts[j], res)
            return res

        def head_tiles(w_buf, t):
            a = t // 4
            r = t % 4
            n32 = M // 4 * H // 2
            sub = w_buf.bitcast(jnp.uint32).at[
                r, pl.ds(pl.multiple_of(4 * a, 4), n32 - 12), :]
            tiles = []
            for u in range(4):
                w = sub[pl.ds(u, 128, stride=H // 2), :]
                even = pltpu.bitcast(w << 16, _F32).astype(_BF16)
                odd = pltpu.bitcast(w & jnp.uint32(0xFFFF0000), _F32).astype(_BF16)
                tiles += [even, odd]
            return a, r, tiles

        def fold(x, op):
            r = x[:, 0:128]
            for t in range(1, x.shape[1] // 128):
                r = op(r, x[:, t * 128:(t + 1) * 128])
            return r

        def qa_task(k):
            w = wq_buf[:, :, k * 1024:(k + 1) * 1024].reshape(M, 1024)
            qa = _dot(x16(xa_buf), w)
            q = pick([qa[:, r * D:(r + 1) * D] for r in range(R)])
            for b in range(B):
                q_scr[b * GPB + k] = q[b * R:(b + 1) * R, :]

        def qk(i):
            g = i // PPG
            j = i % G
            q = q_scr[g].astype(_BF16)
            slot = i % NK
            s = pick([_dot_nt(q, kbuf[slot, r]) for r in range(R)])
            s_scr[:, pl.ds(_mult(j * KP, KP), KP)] = s

        def softmax_update():
            s = s_scr[...]
            m_old = m_scr[:, 0:1]
            m_new = jnp.maximum(m_old, jnp.max(s, axis=1, keepdims=True))
            alpha = jnp.exp((m_old - m_new) * scale)
            p = jnp.exp((s - m_new) * scale)
            l_scr[...] = l_scr[...] * alpha + jnp.sum(p, axis=1, keepdims=True)
            m_scr[...] = jnp.broadcast_to(m_new, (R, D))
            acc_scr[...] = acc_scr[...] * alpha
            p_scr[...] = p.astype(_BF16)

        def pv(i):
            j = i % G
            slot = i % NV
            p = p_scr[:, pl.ds(_mult(j * KP, KP), KP)]
            acc_scr[...] += pick([_dot(p, vbuf[slot, r]) for r in range(R)])

        def reset_group():
            acc_scr[...] = jnp.zeros_like(acc_scr)
            l_scr[...] = jnp.zeros_like(l_scr)
            m_scr[...] = jnp.full(m_scr.shape, -jnp.inf, _F32)

        def finish_group(g):
            o = (acc_scr[...] / l_scr[...]).astype(_BF16)
            hg = g % GPB
            oa_scr[g // GPB] += pick(
                [_dot(o, wo_buf[hg, r * D:(r + 1) * D, :]) for r in range(R)])

        def b_init():
            xb16_scr[...] = x16(xb_buf)
            qb_scr[...] = jnp.zeros_like(qb_scr)
            ctxc_scr[...] = jnp.zeros_like(ctxc_scr)

        def b_query(t):
            a, r, tiles = head_tiles(wqb_buf, t)
            x = xb16_scr[:, pl.ds(_mult(r * 128, 128), 128)]
            qb_scr[a] += pick([_dot(x, w) for w in tiles])

        def b_absorb(t):
            a, r, tiles = head_tiles(wuk_buf, t)
            q = qb_scr[a].astype(_BF16)
            qabs = pick([_dot_nt(q, w) for w in tiles])
            for b in range(B):
                qabs_scr[b, pl.ds(_mult(a * 8, 8), 8),
                         pl.ds(_mult(r * 128, 128), 128)] = qabs[b * 8:(b + 1) * 8, :]

        def b_absorb_done():
            qab_scr[...] = qabs_scr[...].astype(_BF16)
            mb_scr[...] = jnp.full(mb_scr.shape, -jnp.inf, _F32)

        NCB = S // CB
        CPR = 2048 // CB

        def ckv_chunk(t):
            b = t // NCB
            j = t % NCB
            return ckv_buf[b * 4 + j // CPR, pl.ds(_mult((j % CPR) * CB, CB), CB), :]

        def b_scores(t):
            b = t // NCB
            j = t % NCB
            s = _dot_nt(qab_scr[b], ckv_chunk(t))
            sb_scr[b, :, pl.ds(_mult(j * CB, CB), CB)] = s
            mb_scr[b] = jnp.maximum(mb_scr[b], fold(s, jnp.maximum))

        def b_scores_done():
            for b in range(B):
                m = jnp.max(mb_scr[b], axis=1, keepdims=True)
                mb_scr[b] = jnp.broadcast_to(m, (H, 128))
            lb_scr[...] = jnp.zeros_like(lb_scr)
            ctx_scr[...] = jnp.zeros_like(ctx_scr)

        def b_ctx(t):
            b = t // NCB
            j = t % NCB
            s = sb_scr[b, :, pl.ds(_mult(j * CB, CB), CB)]
            p = jnp.exp((s - mb_scr[b][:, 0:1]) * scale)
            lb_scr[b] += fold(p, jnp.add)
            ctx_scr[b] += _dot(p.astype(_BF16), ckv_chunk(t))

        def b_ctx_done():
            for b in range(B):
                ctx_scr[b] = ctx_scr[b] / jnp.sum(lb_scr[b], axis=1, keepdims=True)
            ob_scr[...] = jnp.zeros_like(ob_scr)

        def b_value(t):
            a, r, tiles = head_tiles(wuv_buf, t)
            rows = pl.ds(_mult(a * 8, 8), 8)
            cols = pl.ds(_mult(r * 128, 128), 128)
            lhs = jnp.concatenate(
                [ctx_scr[b, rows, cols] for b in range(B)], axis=0).astype(_BF16)
            ctxc_scr[a] += pick([_dot(lhs, w) for w in tiles])

        def b_out(t):
            a = t // 2
            k0 = (t % 2) * 4
            lhs = ctxc_scr[a].astype(_BF16)
            parts = [
                _dot(lhs, wob_buf[a, pl.ds(_mult((k0 + j) * D, D), D), :])
                for j in range(4)
            ]
            k = lax.broadcasted_iota(jnp.int32, (16, M), 0) % 8
            y = jnp.where(k == k0, parts[0], 0.0)
            for j in range(1, 4):
                y = jnp.where(k == k0 + j, parts[j], y)
            ob_scr[...] += y

        def b_done():
            for b in range(B):
                ob = jnp.sum(ob_scr[b * 8:(b + 1) * 8, :], axis=0, keepdims=True)
                out_ref[b:b + 1, M:2 * M] = ob.astype(out_ref.dtype)

        cp_xa.start()
        cp_xb.start()

        def prologue(it, carry):
            for c in range(P):
                ucp(0, 0, it * P + c).start(priority=_HI)
                ucp(0, 1, it * P + c).start(priority=_LO)
            return carry

        lax.fori_loop(0, BV, prologue, 0)

        def seg_loop(seg, lo, hi, extra=None):
            nxt = lo + BV >= UI

            def body(it, carry):
                for c in range(P):
                    ucp(seg, 1, it * P + c).wait()
                    if not nxt:
                        ucp(seg, 0, (it + BV) * P + c).start(priority=_HI)
                        ucp(seg, 1, (it + BV) * P + c).start(priority=_LO)
                    elif seg + 1 < NSEG:
                        ucp(seg + 1, 0, (it + BV - UI) * P + c).start(priority=_HI)
                        ucp(seg + 1, 1, (it + BV - UI) * P + c).start(priority=_LO)
                    else:
                        kcp(it + BV - UI, c).start(priority=_HI)
                        vcp(it + BV - UI, c).start(priority=_LO)
                    if c == 0 and extra is not None:
                        extra(it)
                return carry

            lax.fori_loop(lo, hi, body, 0)

        for seg in range(NSEG):
            if seg == 1:
                uwait_all(0)
                cp_xa.wait()
                cp_xb.wait()
                for k in range(4):
                    seg_loop(seg, k, k + 1, extra=lambda it, k=k: qa_task(k))
                seg_loop(seg, 4, UI - BV)
            else:
                seg_loop(seg, 0, UI - BV)
            seg_loop(seg, UI - BV, UI)
        for seg in range(1, NSEG):
            uwait_all(seg)

        reset_group()
        oa_scr[...] = jnp.zeros_like(oa_scr)

        def first_block(i, carry):
            kwait_all(i)
            for c in range(P):
                kcp(i + XK, c).start(priority=_HI)
            qk(i)
            return carry

        lax.fori_loop(0, G, first_block, 0)
        softmax_update()
        kwait_all(G)

        def main_loop(lo, hi, extra=None, tail=False):
            def body(i, carry):
                def issue(c):
                    if not tail:
                        kcp(i + G + XK, c).start(priority=_HI)
                        vcp(i + BV, c).start(priority=_LO)
                        return

                    @pl.when(i + G + XK < NP)
                    def _():
                        kcp(i + G + XK, c).start(priority=_HI)

                    if tail_hi and c % 2 == 0:
                        @pl.when(jnp.logical_and(i + BV < NP, i + G + XK < NP))
                        def _():
                            vcp(i + BV, c).start(priority=_LO)

                        @pl.when(jnp.logical_and(i + BV < NP, i + G + XK >= NP))
                        def _():
                            vcp(i + BV, c).start(priority=_HI)
                    else:
                        @pl.when(i + BV < NP)
                        def _():
                            vcp(i + BV, c).start(priority=_LO)

                vcp(i, 0).wait()
                issue(0)
                if tail:
                    @pl.when(i + G < NP)
                    def _():
                        qk(i + G)
                else:
                    qk(i + G)
                if extra is not None:
                    extra(i - lo)
                for c in range(1, P):
                    vcp(i, c).wait()
                    issue(c)
                pv(i)
                if tail:
                    @pl.when(i + G + 1 < NP)
                    def _():
                        kwait_all(i + G + 1)
                else:
                    kwait_all(i + G + 1)

                @pl.when(i % G == G - 1)
                def _():
                    @pl.when(i % PPG == PPG - 1)
                    def _():
                        finish_group(i // PPG)
                        reset_group()

                    if tail:
                        @pl.when(i + 1 < NP)
                        def _():
                            softmax_update()
                    else:
                        softmax_update()

                return carry

            lax.fori_loop(lo, hi, body, 0)

        b_init()
        pos = 0
        for n, task, done in [
            (16, b_query, None),
            (16, b_absorb, b_absorb_done),
            (B * NCB, b_scores, b_scores_done),
            (B * NCB, b_ctx, b_ctx_done),
            (16, b_value, None),
            (8, b_out, b_done),
        ]:
            main_loop(pos, pos + n, extra=task)
            pos += n
            if done is not None:
                done()
        tail0 = NP - 2 * G
        main_loop(pos, tail0)
        main_loop(tail0, NP, tail=True)

        for b in range(B):
            oa = jnp.sum(oa_scr[b], axis=0, keepdims=True)
            out_ref[b:b + 1, 0:M] = oa.astype(out_ref.dtype)

    scratch = [
        pltpu.VMEM((B, M), _BF16),
        pltpu.VMEM((B, M), _BF16),
        pltpu.VMEM((8, 64, HD), _BF16),
        pltpu.VMEM((4, 1024, M), _BF16),
        pltpu.VMEM((4, 4096, D), _BF16),
        pltpu.VMEM((4, 4096, D), _BF16),
        pltpu.VMEM((4, 4096, D), _BF16),
        pltpu.VMEM((4, 1024, M), _BF16),
        pltpu.VMEM((8, 2048, M), _BF16),
        pltpu.VMEM((NK, R, KP, D), _BF16),
        pltpu.VMEM((NV, R, KP, D), _BF16),
        pltpu.VMEM((NG, R, D), _F32),
        pltpu.VMEM((R, KB), _F32),
        pltpu.VMEM((R, KB), _BF16),
        pltpu.VMEM((R, D), _F32),
        pltpu.VMEM((R, D), _F32),
        pltpu.VMEM((R, D), _F32),
        pltpu.VMEM((B, R, M), _F32),
        pltpu.VMEM((16, M), _BF16),
        pltpu.VMEM((GPB, 16, D), _F32),
        pltpu.VMEM((B, H, M), _F32),
        pltpu.VMEM((B, H, M), _BF16),
        pltpu.VMEM((B, H, S), _F32),
        pltpu.VMEM((B, H, 128), _F32),
        pltpu.VMEM((B, H, 128), _F32),
        pltpu.VMEM((B, H, M), _F32),
        pltpu.VMEM((GPB, 16, D), _F32),
        pltpu.VMEM((16, M), _F32),
        pltpu.SemaphoreType.DMA((2,)),
        pltpu.SemaphoreType.DMA((10,)),
        pltpu.SemaphoreType.DMA((NK,)),
        pltpu.SemaphoreType.DMA((NV,)),
    ]

    def call(A_x, A_k_cache, A_v_cache, A_wq, A_wo, B_x, B_c_kv, B_w_q, B_w_uk,
             B_w_uv, B_w_o):
        any_spec = pl.BlockSpec(memory_space=pl.ANY)
        out = pl.pallas_call(
            kernel,
            out_shape=jax.ShapeDtypeStruct((B, 2 * M), _BF16),
            in_specs=[any_spec] * 11,
            out_specs=pl.BlockSpec(memory_space=pltpu.VMEM),
            scratch_shapes=scratch,
            compiler_params=pltpu.CompilerParams(
                vmem_limit_bytes=100 * 1024 * 1024,
                disable_bounds_checks=True),
        )(
            A_x.reshape(B, M),
            A_k_cache.reshape(NBH, S, D),
            A_v_cache.reshape(NBH, S, D),
            A_wq.reshape(8, 64, HD),
            A_wo.reshape(4, 1024, M),
            B_x.reshape(B, M),
            B_c_kv.reshape(8, 2048, M),
            B_w_q.reshape(4, 4096, D),
            B_w_uk.reshape(4, 4096, D),
            B_w_uv.reshape(4, 4096, D),
            B_w_o.reshape(4, 1024, M),
        )
        return out.reshape(B, 1, 2 * M)

    return call


@jax.jit
def pallas_concat_heads__gqa_block_cached__compressed_kv_cla__decode_kernel(
    A_x: jax.Array,
    A_k_cache: jax.Array,
    A_v_cache: jax.Array,
    A_wq: jax.Array,
    A_wo: jax.Array,
    B_x: jax.Array,
    B_c_kv: jax.Array,
    B_w_q: jax.Array,
    B_w_uk: jax.Array,
    B_w_uv: jax.Array,
    B_w_o: jax.Array,
):
    B, H, S, D = A_k_cache.shape
    M = A_x.shape[-1]
    assert A_x.shape == (B, 1, M) and B_x.shape == (B, 1, M)
    assert A_wq.shape == (M, H * D) and B_c_kv.shape == (B, S, M)
    assert B_w_q.shape == (M, H, D) and B_w_o.shape == (H, D, M)
    return _build(B, H, S, D, M)(A_x, A_k_cache, A_v_cache, A_wq, A_wo, B_x,
                                 B_c_kv, B_w_q, B_w_uk, B_w_uv, B_w_o)
```

```python
import functools

import jax
import jax.numpy as jnp
from jax import lax
import jax.experimental.pallas as pl
import jax.experimental.pallas.tpu as pltpu

_NT = (((1,), (1,)), ((), ()))
_BF16 = jnp.bfloat16
_F32 = jnp.float32
_HI, _LO = 0, 1


def _dot(a, b):
    return jnp.dot(a, b, preferred_element_type=_F32)


def _dot_nt(a, b):
    return lax.dot_general(a, b, _NT, preferred_element_type=_F32)


def _mult(x, m):
    return x if isinstance(x, int) else pl.multiple_of(x, m)


def _build(B, H, S, D, M, XK=6, BV=6, KB=512, CB=256):
    R = 8
    C = 16
    KP = 128
    P = KP // C
    G = KB // KP
    PPG = S // KP
    NBH = B * H
    GPB = H // R
    NG = NBH // R
    NP = NG * PPG
    NK = XK + 2
    NV = BV + 2
    HD = H * D
    scale = float(D) ** -0.5
    UD = 128
    UI = UD // P
    assert XK == BV and BV < UI
    assert M == 512 and D == 128 and HD == 4096 and B == 2

    def kernel(xa_hbm, k_hbm, v_hbm, wq_hbm, wo_hbm, xb_hbm, ckv_hbm, wqb_hbm,
               wuk_hbm, wuv_hbm, wob_hbm, out_ref,
               xa_buf, xb_buf, wq_buf, wo_buf, wqb_buf, wuk_buf, wuv_buf, wob_buf,
               ckv_buf, kbuf, vbuf, q_scr, s_scr, p_scr, m_scr, l_scr, acc_scr,
               oa_scr, xb16_scr, qb_scr, qabs_scr, qab_scr, sb_scr, mb_scr, lb_scr, ctx_scr,
               ctxc_scr, ob_scr):
        pl.run_scoped(
            functools.partial(
                body_fn, xa_hbm, k_hbm, v_hbm, wq_hbm, wo_hbm, xb_hbm, ckv_hbm,
                wqb_hbm, wuk_hbm, wuv_hbm, wob_hbm, out_ref,
                xa_buf, xb_buf, wq_buf, wo_buf, wqb_buf, wuk_buf, wuv_buf, wob_buf,
                ckv_buf, kbuf, vbuf, q_scr, s_scr, p_scr, m_scr, l_scr, acc_scr,
                oa_scr, xb16_scr, qb_scr, qabs_scr, qab_scr, sb_scr, mb_scr, lb_scr,
                ctx_scr, ctxc_scr, ob_scr),
            pltpu.SemaphoreType.DMA((2,)),
            pltpu.SemaphoreType.DMA((10,)),
            pltpu.SemaphoreType.DMA((NK,)),
            pltpu.SemaphoreType.DMA((NV,)),
        )

    def body_fn(xa_hbm, k_hbm, v_hbm, wq_hbm, wo_hbm, xb_hbm, ckv_hbm, wqb_hbm,
                wuk_hbm, wuv_hbm, wob_hbm, out_ref,
                xa_buf, xb_buf, wq_buf, wo_buf, wqb_buf, wuk_buf, wuv_buf, wob_buf,
                ckv_buf, kbuf, vbuf, q_scr, s_scr, p_scr, m_scr, l_scr, acc_scr,
                oa_scr, xb16_scr, qb_scr, qabs_scr, qab_scr, sb_scr, mb_scr, lb_scr,
                ctx_scr, ctxc_scr, ob_scr, semx, semu, semk, semv):
        cp_xa = pltpu.make_async_copy(xa_hbm, xa_buf, semx.at[0])
        cp_xb = pltpu.make_async_copy(xb_hbm, xb_buf, semx.at[1])

        def unit_wq(j):
            idx = (slice(None), pl.ds(_mult((j // 16) * 8, 8), 8),
                   pl.ds(_mult((j % 16) * 256, 256), 256))
            return wq_hbm.at[idx], wq_buf.at[idx]

        def unit_rows(hbm, buf):
            def f(j):
                idx = (slice(None), pl.ds(_mult(j * 32, 32), 32), slice(None))
                return hbm.at[idx], buf.at[idx]
            return f

        def unit_wide(hbm, buf, r0=0, row0=0):
            def f(j):
                idx = (pl.ds(r0, 4), pl.ds(_mult(row0 + j * 8, 8), 8), slice(None))
                return hbm.at[idx], buf.at[idx]
            return f

        segs = [
            (unit_wq, unit_rows(wqb_hbm, wqb_buf)),
            (unit_rows(wuk_hbm, wuk_buf), unit_wide(ckv_hbm, ckv_buf, 0, 0)),
            (unit_wide(ckv_hbm, ckv_buf, 0, 1024), unit_wide(ckv_hbm, ckv_buf, 4, 0)),
            (unit_wide(ckv_hbm, ckv_buf, 4, 1024), unit_rows(wuv_hbm, wuv_buf)),
            (unit_wide(wo_hbm, wo_buf), unit_wide(wob_hbm, wob_buf)),
        ]
        NSEG = len(segs)

        def ucp(seg, side, j):
            src, dst = segs[seg][side](j)
            return pltpu.make_async_copy(src, dst, semu.at[2 * seg + side])

        hi_dst = [wq_buf, wuk_buf, ckv_buf.at[pl.ds(0, 4), pl.ds(1024, 1024), :],
                  ckv_buf.at[pl.ds(4, 4), pl.ds(1024, 1024), :], wo_buf]

        def uwait_all(seg):
            pltpu.make_async_copy(hi_dst[seg], hi_dst[seg], semu.at[2 * seg]).wait()

        def kv_src(hbm, i, c):
            g = i // PPG
            j = i % PPG
            return hbm.at[pl.ds(g * R, R), pl.ds(_mult(j * KP + c * C, C), C), :]

        def kcp(i, c):
            slot = i % NK
            return pltpu.make_async_copy(
                kv_src(k_hbm, i, c), kbuf.at[slot, :, pl.ds(c * C, C), :],
                semk.at[slot])

        def vcp(i, c):
            slot = i % NV
            return pltpu.make_async_copy(
                kv_src(v_hbm, i, c), vbuf.at[slot, :, pl.ds(c * C, C), :],
                semv.at[slot])

        HPP = R // G

        def vcp_last(i, c):
            u = i - (NP - G)
            slot = i % NV
            head = (NG - 1) * R + u * HPP + c // G
            key0 = S - KB + (c % G) * KP
            return pltpu.make_async_copy(
                v_hbm.at[head, pl.ds(key0, KP), :], vbuf.at[slot, c], semv.at[slot])

        def kwait_all(i):
            slot = i % NK
            pltpu.make_async_copy(kbuf.at[slot], kbuf.at[slot], semk.at[slot]).wait()

        def x16(buf):
            x = buf[...].astype(_F32)
            row = lax.broadcasted_iota(jnp.int32, (16, M), 0)
            z = jnp.where(row < 8, jnp.broadcast_to(x[0:1, :], (16, M)),
                          jnp.broadcast_to(x[1:2, :], (16, M)))
            return z.astype(_BF16)

        def pick(parts, k0=0):
            shape = parts[0].shape
            k = lax.broadcasted_iota(jnp.int32, shape, 0) % 8
            res = parts[0]
            for j in range(1, len(parts)):
                res = jnp.where(k == k0 + j, parts[j], res)
            return res

        def head_tiles(w_buf, t):
            a = t // 4
            r = t % 4
            n32 = M // 4 * H // 2
            sub = w_buf.bitcast(jnp.uint32).at[
                r, pl.ds(pl.multiple_of(4 * a, 4), n32 - 12), :]
            tiles = []
            for u in range(4):
                w = sub[pl.ds(u, 128, stride=H // 2), :]
                even = pltpu.bitcast(w << 16, _F32).astype(_BF16)
                odd = pltpu.bitcast(w & jnp.uint32(0xFFFF0000), _F32).astype(_BF16)
                tiles += [even, odd]
            return a, r, tiles

        def fold(x, op):
            r = x[:, 0:128]
            for t in range(1, x.shape[1] // 128):
                r = op(r, x[:, t * 128:(t + 1) * 128])
            return r

        def qa_task(k):
            w = wq_buf[:, :, k * 1024:(k + 1) * 1024].reshape(M, 1024)
            qa = _dot(x16(xa_buf), w)
            q = pick([qa[:, r * D:(r + 1) * D] for r in range(R)])
            for b in range(B):
                q_scr[b * GPB + k] = q[b * R:(b + 1) * R, :]

        def qk(i):
            g = i // PPG
            j = i % G
            q = q_scr[g].astype(_BF16)
            slot = i % NK
            s = pick([_dot_nt(q, kbuf[slot, r]) for r in range(R)])
            s_scr[:, pl.ds(_mult(j * KP, KP), KP)] = s

        def softmax_update():
            s = [s_scr[:, t * 128:(t + 1) * 128] for t in range(KB // 128)]
            mx = functools.reduce(jnp.maximum, s)
            m_old = m_scr[...]
            m_new = jnp.maximum(m_old, jnp.max(mx, axis=1, keepdims=True))
            alpha = jnp.exp((m_old - m_new) * scale)
            p = [jnp.exp((st - m_new) * scale) for st in s]
            l_scr[...] = l_scr[...] * alpha + functools.reduce(jnp.add, p)
            m_scr[...] = m_new
            acc_scr[...] = acc_scr[...] * alpha
            for t in range(KB // 128):
                p_scr[:, t * 128:(t + 1) * 128] = p[t].astype(_BF16)

        def inv_l():
            return 1.0 / jnp.sum(l_scr[...], axis=1, keepdims=True)

        def pv(i):
            j = i % G
            slot = i % NV
            p = p_scr[:, pl.ds(_mult(j * KP, KP), KP)]
            acc_scr[...] += pick([_dot(p, vbuf[slot, r]) for r in range(R)])

        def reset_group():
            acc_scr[...] = jnp.zeros_like(acc_scr)
            l_scr[...] = jnp.zeros_like(l_scr)
            m_scr[...] = jnp.full(m_scr.shape, -jnp.inf, _F32)

        def finish_group(g):
            o = (acc_scr[...] * inv_l()).astype(_BF16)
            hg = g % GPB
            oa_scr[g // GPB] += pick(
                [_dot(o, wo_buf[hg, r * D:(r + 1) * D, :]) for r in range(R)])

        def b_init():
            xb16_scr[...] = x16(xb_buf)
            qb_scr[...] = jnp.zeros_like(qb_scr)
            ctxc_scr[...] = jnp.zeros_like(ctxc_scr)

        def b_query(t):
            a, r, tiles = head_tiles(wqb_buf, t)
            x = xb16_scr[:, pl.ds(_mult(r * 128, 128), 128)]
            qb_scr[a] += pick([_dot(x, w) for w in tiles])

        def b_absorb(t):
            a, r, tiles = head_tiles(wuk_buf, t)
            q = qb_scr[a].astype(_BF16)
            qabs = pick([_dot_nt(q, w) for w in tiles])
            for b in range(B):
                qabs_scr[b, pl.ds(_mult(a * 8, 8), 8),
                         pl.ds(_mult(r * 128, 128), 128)] = qabs[b * 8:(b + 1) * 8, :]

        def b_absorb_done():
            qab_scr[...] = qabs_scr[...].astype(_BF16)
            mb_scr[...] = jnp.full(mb_scr.shape, -jnp.inf, _F32)

        NCB = S // CB
        CPR = 2048 // CB

        def ckv_chunk(t):
            b = t // NCB
            j = t % NCB
            return ckv_buf[b * 4 + j // CPR, pl.ds(_mult((j % CPR) * CB, CB), CB), :]

        def b_scores(t):
            b = t // NCB
            j = t % NCB
            s = _dot_nt(qab_scr[b], ckv_chunk(t))
            sb_scr[b, :, pl.ds(_mult(j * CB, CB), CB)] = s
            mb_scr[b] = jnp.maximum(mb_scr[b], fold(s, jnp.maximum))

        def b_scores_done():
            for b in range(B):
                m = jnp.max(mb_scr[b], axis=1, keepdims=True)
                mb_scr[b] = jnp.broadcast_to(m, (H, 128))
            lb_scr[...] = jnp.zeros_like(lb_scr)
            ctx_scr[...] = jnp.zeros_like(ctx_scr)

        def b_ctx(t):
            b = t // NCB
            j = t % NCB
            s = sb_scr[b, :, pl.ds(_mult(j * CB, CB), CB)]
            m = mb_scr[b]
            p = jnp.concatenate(
                [jnp.exp((s[:, u * 128:(u + 1) * 128] - m) * scale)
                 for u in range(CB // 128)], axis=1)
            lb_scr[b] += fold(p, jnp.add)
            ctx_scr[b] += _dot(p.astype(_BF16), ckv_chunk(t))

        def b_ctx_done():
            for b in range(B):
                ctx_scr[b] = ctx_scr[b] / jnp.sum(lb_scr[b], axis=1, keepdims=True)
            ob_scr[...] = jnp.zeros_like(ob_scr)

        def b_value(t):
            a, r, tiles = head_tiles(wuv_buf, t)
            rows = pl.ds(_mult(a * 8, 8), 8)
            cols = pl.ds(_mult(r * 128, 128), 128)
            lhs = jnp.concatenate(
                [ctx_scr[b, rows, cols] for b in range(B)], axis=0).astype(_BF16)
            ctxc_scr[a] += pick([_dot(lhs, w) for w in tiles])

        def b_out(t):
            a = t // 2
            k0 = (t % 2) * 4
            lhs = ctxc_scr[a].astype(_BF16)
            parts = [
                _dot(lhs, wob_buf[a, pl.ds(_mult((k0 + j) * D, D), D), :])
                for j in range(4)
            ]
            k = lax.broadcasted_iota(jnp.int32, (16, M), 0) % 8
            y = jnp.where(k == k0, parts[0], 0.0)
            for j in range(1, 4):
                y = jnp.where(k == k0 + j, parts[j], y)
            ob_scr[...] += y

        def b_done():
            for b in range(B):
                ob = jnp.sum(ob_scr[b * 8:(b + 1) * 8, :], axis=0, keepdims=True)
                out_ref[b:b + 1, M:2 * M] = ob.astype(out_ref.dtype)

        cp_xa.start()
        cp_xb.start()

        def prologue(it, carry):
            for c in range(P):
                ucp(0, 0, it * P + c).start(priority=_HI)
                ucp(0, 1, it * P + c).start(priority=_LO)
            return carry

        lax.fori_loop(0, BV, prologue, 0)

        def seg_loop(seg, lo, hi, extra=None):
            nxt = lo + BV >= UI

            def body(it, carry):
                for c in range(P):
                    ucp(seg, 1, it * P + c).wait()
                    if not nxt:
                        ucp(seg, 0, (it + BV) * P + c).start(priority=_HI)
                        ucp(seg, 1, (it + BV) * P + c).start(priority=_LO)
                    elif seg + 1 < NSEG:
                        ucp(seg + 1, 0, (it + BV - UI) * P + c).start(priority=_HI)
                        ucp(seg + 1, 1, (it + BV - UI) * P + c).start(priority=_LO)
                    else:
                        kcp(it + BV - UI, c).start(priority=_HI)
                        vcp(it + BV - UI, c).start(priority=_LO)
                    if c == 0 and extra is not None:
                        extra(it)
                return carry

            lax.fori_loop(lo, hi, body, 0)

        for seg in range(NSEG):
            if seg == 1:
                uwait_all(0)
                cp_xa.wait()
                cp_xb.wait()
                for k in range(4):
                    seg_loop(seg, k, k + 1, extra=lambda it, k=k: qa_task(k))
                seg_loop(seg, 4, UI - BV)
            else:
                seg_loop(seg, 0, UI - BV)
            seg_loop(seg, UI - BV, UI)
        for seg in range(1, NSEG):
            uwait_all(seg)

        reset_group()
        oa_scr[...] = jnp.zeros_like(oa_scr)

        def first_block(i, carry):
            kwait_all(i)
            for c in range(P):
                kcp(i + XK, c).start(priority=_HI)
            qk(i)
            return carry

        lax.fori_loop(0, G, first_block, 0)
        softmax_update()
        kwait_all(G)

        def end_of_piece(i):
            @pl.when(i % G == G - 1)
            def _():
                @pl.when(i % PPG == PPG - 1)
                def _():
                    finish_group(i // PPG)
                    reset_group()

                softmax_update()

        def main_loop(lo, hi, extra=None):
            def body(i, carry):
                def issue(c):
                    kcp(i + G + XK, c).start(priority=_HI)
                    vcp(i + BV, c).start(priority=_LO)

                vcp(i, 0).wait()
                issue(0)
                qk(i + G)
                if extra is not None:
                    extra(i - lo)
                for c in range(1, P):
                    vcp(i, c).wait()
                    issue(c)
                pv(i)
                kwait_all(i + G + 1)
                end_of_piece(i)
                return carry

            lax.fori_loop(lo, hi, body, 0)

        def tail_loop(lo, hi):
            def body(i, carry):
                for c in range(P):
                    vcp(i, c).wait()

                    @pl.when(i + BV < NP - G)
                    def _():
                        vcp(i + BV, c).start(priority=_LO)

                    @pl.when(jnp.logical_and(i + BV >= NP - G, i + BV < NP))
                    def _():
                        vcp_last(i + BV, c).start(priority=_LO)

                qk(i + G)
                pv(i)

                @pl.when(i + G + 1 < NP)
                def _():
                    kwait_all(i + G + 1)

                end_of_piece(i)
                return carry

            lax.fori_loop(lo, hi, body, 0)

        def last_block():
            g = NG - 1
            row = lax.broadcasted_iota(jnp.int32, (R, M), 0)
            rl = inv_l()
            y = oa_scr[B - 1]
            for u in range(G):
                i = NP - G + u
                for c in range(P):
                    vcp_last(i, c).wait()
                    if i + BV < NP:
                        vcp_last(i + BV, c).start(priority=_LO)
                slot = i % NV
                rowd = lax.broadcasted_iota(jnp.int32, (R, D), 0)
                o = None
                for e in range(HPP):
                    oe = functools.reduce(jnp.add, [
                        _dot(p_scr[:, kt * KP:(kt + 1) * KP], vbuf[slot, e * G + kt])
                        for kt in range(G)])
                    o = oe if o is None else jnp.where(rowd == u * HPP + e, oe, o)
                o = ((acc_scr[...] + o) * rl).astype(_BF16)
                for e in range(HPP):
                    r = u * HPP + e
                    yr = _dot(o, wo_buf[g % GPB, r * D:(r + 1) * D, :])
                    y = y + jnp.where(row == r, yr, 0.0)
            out_ref[B - 1:B, 0:M] = jnp.sum(y, axis=0, keepdims=True).astype(out_ref.dtype)

        b_init()
        pos = 0
        for n, task, done in [
            (16, b_query, None),
            (16, b_absorb, b_absorb_done),
            (B * NCB, b_scores, b_scores_done),
            (B * NCB, b_ctx, b_ctx_done),
            (16, b_value, None),
            (8, b_out, b_done),
        ]:
            main_loop(pos, pos + n, extra=task)
            pos += n
            if done is not None:
                done()
        tail0 = NP - G - XK
        assert XK >= BV
        assert pos <= tail0 and P % G == 0 and HPP * G == R and P == R
        main_loop(pos, tail0)
        for b in range(B - 1):
            oa = jnp.sum(oa_scr[b], axis=0, keepdims=True)
            out_ref[b:b + 1, 0:M] = oa.astype(out_ref.dtype)
        tail_loop(tail0, NP - G)
        last_block()

    scratch = [
        pltpu.VMEM((B, M), _BF16),
        pltpu.VMEM((B, M), _BF16),
        pltpu.VMEM((8, 64, HD), _BF16),
        pltpu.VMEM((4, 1024, M), _BF16),
        pltpu.VMEM((4, 4096, D), _BF16),
        pltpu.VMEM((4, 4096, D), _BF16),
        pltpu.VMEM((4, 4096, D), _BF16),
        pltpu.VMEM((4, 1024, M), _BF16),
        pltpu.VMEM((8, 2048, M), _BF16),
        pltpu.VMEM((NK, R, KP, D), _BF16),
        pltpu.VMEM((NV, R, KP, D), _BF16),
        pltpu.VMEM((NG, R, D), _F32),
        pltpu.VMEM((R, KB), _F32),
        pltpu.VMEM((R, KB), _BF16),
        pltpu.VMEM((R, D), _F32),
        pltpu.VMEM((R, D), _F32),
        pltpu.VMEM((R, D), _F32),
        pltpu.VMEM((B, R, M), _F32),
        pltpu.VMEM((16, M), _BF16),
        pltpu.VMEM((GPB, 16, D), _F32),
        pltpu.VMEM((B, H, M), _F32),
        pltpu.VMEM((B, H, M), _BF16),
        pltpu.VMEM((B, H, S), _F32),
        pltpu.VMEM((B, H, 128), _F32),
        pltpu.VMEM((B, H, 128), _F32),
        pltpu.VMEM((B, H, M), _F32),
        pltpu.VMEM((GPB, 16, D), _F32),
        pltpu.VMEM((16, M), _F32),
    ]

    def call(A_x, A_k_cache, A_v_cache, A_wq, A_wo, B_x, B_c_kv, B_w_q, B_w_uk,
             B_w_uv, B_w_o):
        any_spec = pl.BlockSpec(memory_space=pl.ANY)
        out = pl.pallas_call(
            kernel,
            out_shape=jax.ShapeDtypeStruct((B, 2 * M), _BF16),
            in_specs=[any_spec] * 11,
            out_specs=pl.BlockSpec(memory_space=pltpu.VMEM),
            scratch_shapes=scratch,
            compiler_params=pltpu.CompilerParams(
                vmem_limit_bytes=100 * 1024 * 1024,
                disable_bounds_checks=True),
        )(
            A_x.reshape(B, M),
            A_k_cache.reshape(NBH, S, D),
            A_v_cache.reshape(NBH, S, D),
            A_wq.reshape(8, 64, HD),
            A_wo.reshape(4, 1024, M),
            B_x.reshape(B, M),
            B_c_kv.reshape(8, 2048, M),
            B_w_q.reshape(4, 4096, D),
            B_w_uk.reshape(4, 4096, D),
            B_w_uv.reshape(4, 4096, D),
            B_w_o.reshape(4, 1024, M),
        )
        return out.reshape(B, 1, 2 * M)

    return call


@jax.jit
def pallas_concat_heads__gqa_block_cached__compressed_kv_cla__decode_kernel(
    A_x: jax.Array,
    A_k_cache: jax.Array,
    A_v_cache: jax.Array,
    A_wq: jax.Array,
    A_wo: jax.Array,
    B_x: jax.Array,
    B_c_kv: jax.Array,
    B_w_q: jax.Array,
    B_w_uk: jax.Array,
    B_w_uv: jax.Array,
    B_w_o: jax.Array,
):
    B, H, S, D = A_k_cache.shape
    M = A_x.shape[-1]
    assert A_x.shape == (B, 1, M) and B_x.shape == (B, 1, M)
    assert A_wq.shape == (M, H * D) and B_c_kv.shape == (B, S, M)
    assert B_w_q.shape == (M, H, D) and B_w_o.shape == (H, D, M)
    return _build(B, H, S, D, M)(A_x, A_k_cache, A_v_cache, A_wq, A_wo, B_x,
                                 B_c_kv, B_w_q, B_w_uk, B_w_uv, B_w_o)
```

```python
import functools

import jax
import jax.numpy as jnp
from jax import lax
import jax.experimental.pallas as pl
import jax.experimental.pallas.tpu as pltpu

_NT = (((1,), (1,)), ((), ()))
_BF16 = jnp.bfloat16
_F32 = jnp.float32
_HI, _LO = 0, 1


def _dot(a, b):
    return jnp.dot(a, b, preferred_element_type=_F32)


def _dot_nt(a, b):
    return lax.dot_general(a, b, _NT, preferred_element_type=_F32)


def _mult(x, m):
    return x if isinstance(x, int) else pl.multiple_of(x, m)


def _build(B, H, S, D, M, XK=6, BV=6, KB=512, CB=256):
    R = 8
    C = 16
    KP = 128
    P = KP // C
    G = KB // KP
    PPG = S // KP
    NBH = B * H
    GPB = H // R
    NG = NBH // R
    NP = NG * PPG
    NK = XK + 2
    NV = BV + 2
    HD = H * D
    scale = float(D) ** -0.5
    UD = 128
    UI = UD // P
    assert XK == BV and BV < UI
    assert M == 512 and D == 128 and HD == 4096 and B == 2

    def kernel(xa_hbm, k_hbm, v_hbm, wq_hbm, wo_hbm, xb_hbm, ckv_hbm, wqb_hbm,
               wuk_hbm, wuv_hbm, wob_hbm, out_ref,
               xa_buf, xb_buf, wq_buf, wo_buf, wqb_buf, wuk_buf, wuv_buf, wob_buf,
               ckv_buf, kbuf, vbuf, q_scr, s_scr, p_scr, m_scr, l_scr, acc_scr,
               oa_scr, xb16_scr, qb_scr, qabs_scr, qab_scr, sb_scr, mb_scr, lb_scr, ctx_scr,
               ctxc_scr, ob_scr):
        pl.run_scoped(
            functools.partial(
                body_fn, xa_hbm, k_hbm, v_hbm, wq_hbm, wo_hbm, xb_hbm, ckv_hbm,
                wqb_hbm, wuk_hbm, wuv_hbm, wob_hbm, out_ref,
                xa_buf, xb_buf, wq_buf, wo_buf, wqb_buf, wuk_buf, wuv_buf, wob_buf,
                ckv_buf, kbuf, vbuf, q_scr, s_scr, p_scr, m_scr, l_scr, acc_scr,
                oa_scr, xb16_scr, qb_scr, qabs_scr, qab_scr, sb_scr, mb_scr, lb_scr,
                ctx_scr, ctxc_scr, ob_scr),
            pltpu.SemaphoreType.DMA((2,)),
            pltpu.SemaphoreType.DMA((10,)),
            pltpu.SemaphoreType.DMA((NK,)),
            pltpu.SemaphoreType.DMA((NV,)),
        )

    def body_fn(xa_hbm, k_hbm, v_hbm, wq_hbm, wo_hbm, xb_hbm, ckv_hbm, wqb_hbm,
                wuk_hbm, wuv_hbm, wob_hbm, out_ref,
                xa_buf, xb_buf, wq_buf, wo_buf, wqb_buf, wuk_buf, wuv_buf, wob_buf,
                ckv_buf, kbuf, vbuf, q_scr, s_scr, p_scr, m_scr, l_scr, acc_scr,
                oa_scr, xb16_scr, qb_scr, qabs_scr, qab_scr, sb_scr, mb_scr, lb_scr,
                ctx_scr, ctxc_scr, ob_scr, semx, semu, semk, semv):
        cp_xa = pltpu.make_async_copy(xa_hbm, xa_buf, semx.at[0])
        cp_xb = pltpu.make_async_copy(xb_hbm, xb_buf, semx.at[1])

        def unit_wq(j):
            idx = (slice(None), pl.ds(_mult((j // 16) * 8, 8), 8),
                   pl.ds(_mult((j % 16) * 256, 256), 256))
            return wq_hbm.at[idx], wq_buf.at[idx]

        def unit_rows(hbm, buf):
            def f(j):
                idx = (slice(None), pl.ds(_mult(j * 32, 32), 32), slice(None))
                return hbm.at[idx], buf.at[idx]
            return f

        def unit_wide(hbm, buf):
            def f(j):
                idx = (slice(None), pl.ds(_mult(j * 8, 8), 8), slice(None))
                return hbm.at[idx], buf.at[idx]
            return f

        def unit_ckv(u):
            def f(j):
                idx = (slice(None), pl.ds(_mult(u * 512 + (j // 2) * 8, 8), 8),
                       pl.ds(_mult((j % 2) * 256, 256), 256))
                return ckv_hbm.at[idx], ckv_buf.at[idx]
            return f

        segs = [
            (unit_wq, unit_rows(wqb_hbm, wqb_buf)),
            (unit_ckv(0), unit_rows(wuk_hbm, wuk_buf)),
            (unit_ckv(1), unit_rows(wuv_hbm, wuv_buf)),
            (unit_ckv(2), unit_wide(wo_hbm, wo_buf)),
            (unit_ckv(3), unit_wide(wob_hbm, wob_buf)),
        ]
        NSEG = len(segs)

        def ucp(seg, side, j):
            src, dst = segs[seg][side](j)
            return pltpu.make_async_copy(src, dst, semu.at[2 * seg + side])

        hi_dst = [wq_buf] + [ckv_buf.at[:, pl.ds(u * 512, 512), :] for u in range(4)]

        def uwait_all(seg):
            pltpu.make_async_copy(hi_dst[seg], hi_dst[seg], semu.at[2 * seg]).wait()

        def kv_src(hbm, i, c):
            g = i // PPG
            j = i % PPG
            return hbm.at[pl.ds(g * R, R), pl.ds(_mult(j * KP + c * C, C), C), :]

        def kcp(i, c):
            slot = i % NK
            return pltpu.make_async_copy(
                kv_src(k_hbm, i, c), kbuf.at[slot, :, pl.ds(c * C, C), :],
                semk.at[slot])

        def vcp(i, c):
            slot = i % NV
            return pltpu.make_async_copy(
                kv_src(v_hbm, i, c), vbuf.at[slot, :, pl.ds(c * C, C), :],
                semv.at[slot])

        HPP = R // G

        def vcp_last(i, c):
            u = i - (NP - G)
            slot = i % NV
            head = (NG - 1) * R + u * HPP + c // G
            key0 = S - KB + (c % G) * KP
            return pltpu.make_async_copy(
                v_hbm.at[head, pl.ds(key0, KP), :], vbuf.at[slot, c], semv.at[slot])

        def kwait_all(i):
            slot = i % NK
            pltpu.make_async_copy(kbuf.at[slot], kbuf.at[slot], semk.at[slot]).wait()

        def x16(buf):
            x = buf[...].astype(_F32)
            row = lax.broadcasted_iota(jnp.int32, (16, M), 0)
            z = jnp.where(row < 8, jnp.broadcast_to(x[0:1, :], (16, M)),
                          jnp.broadcast_to(x[1:2, :], (16, M)))
            return z.astype(_BF16)

        def pick(parts, k0=0):
            shape = parts[0].shape
            k = lax.broadcasted_iota(jnp.int32, shape, 0) % 8
            res = parts[0]
            for j in range(1, len(parts)):
                res = jnp.where(k == k0 + j, parts[j], res)
            return res

        def head_tiles(w_buf, t):
            a = t // 4
            r = t % 4
            n32 = M // 4 * H // 2
            sub = w_buf.bitcast(jnp.uint32).at[
                r, pl.ds(pl.multiple_of(4 * a, 4), n32 - 12), :]
            tiles = []
            for u in range(4):
                w = sub[pl.ds(u, 128, stride=H // 2), :]
                even = pltpu.bitcast(w << 16, _F32).astype(_BF16)
                odd = pltpu.bitcast(w & jnp.uint32(0xFFFF0000), _F32).astype(_BF16)
                tiles += [even, odd]
            return a, r, tiles

        def fold(x, op):
            r = x[:, 0:128]
            for t in range(1, x.shape[1] // 128):
                r = op(r, x[:, t * 128:(t + 1) * 128])
            return r

        def qa_task(k):
            w = wq_buf[:, :, k * 1024:(k + 1) * 1024].reshape(M, 1024)
            qa = _dot(x16(xa_buf), w)
            q = pick([qa[:, r * D:(r + 1) * D] for r in range(R)])
            for b in range(B):
                q_scr[b * GPB + k] = q[b * R:(b + 1) * R, :]

        def qk(i):
            g = i // PPG
            j = i % G
            q = q_scr[g].astype(_BF16)
            slot = i % NK
            s = pick([_dot_nt(q, kbuf[slot, r]) for r in range(R)])
            s_scr[:, pl.ds(_mult(j * KP, KP), KP)] = s

        def softmax_update():
            s = [s_scr[:, t * 128:(t + 1) * 128] for t in range(KB // 128)]
            mx = functools.reduce(jnp.maximum, s)
            m_old = m_scr[...]
            m_new = jnp.maximum(m_old, jnp.max(mx, axis=1, keepdims=True))
            alpha = jnp.exp((m_old - m_new) * scale)
            p = [jnp.exp((st - m_new) * scale) for st in s]
            l_scr[...] = l_scr[...] * alpha + functools.reduce(jnp.add, p)
            m_scr[...] = m_new
            acc_scr[...] = acc_scr[...] * alpha
            for t in range(KB // 128):
                p_scr[:, t * 128:(t + 1) * 128] = p[t].astype(_BF16)

        def inv_l():
            return 1.0 / jnp.sum(l_scr[...], axis=1, keepdims=True)

        def pv(i):
            j = i % G
            slot = i % NV
            p = p_scr[:, pl.ds(_mult(j * KP, KP), KP)]
            acc_scr[...] += pick([_dot(p, vbuf[slot, r]) for r in range(R)])

        def reset_group():
            acc_scr[...] = jnp.zeros_like(acc_scr)
            l_scr[...] = jnp.zeros_like(l_scr)
            m_scr[...] = jnp.full(m_scr.shape, -jnp.inf, _F32)

        def finish_group(g):
            o = (acc_scr[...] * inv_l()).astype(_BF16)
            hg = g % GPB
            oa_scr[g // GPB] += pick(
                [_dot(o, wo_buf[hg, r * D:(r + 1) * D, :]) for r in range(R)])

        def b_init():
            xb16_scr[...] = x16(xb_buf)
            qb_scr[...] = jnp.zeros_like(qb_scr)
            ctxc_scr[...] = jnp.zeros_like(ctxc_scr)

        def b_query(t):
            a, r, tiles = head_tiles(wqb_buf, t)
            x = xb16_scr[:, pl.ds(_mult(r * 128, 128), 128)]
            qb_scr[a] += pick([_dot(x, w) for w in tiles])

        def b_absorb(t):
            a, r, tiles = head_tiles(wuk_buf, t)
            q = qb_scr[a].astype(_BF16)
            qabs = pick([_dot_nt(q, w) for w in tiles])
            for b in range(B):
                qabs_scr[b, pl.ds(_mult(a * 8, 8), 8),
                         pl.ds(_mult(r * 128, 128), 128)] = qabs[b * 8:(b + 1) * 8, :]

        def b_absorb_done():
            qab_scr[...] = qabs_scr[...].astype(_BF16)
            mb_scr[...] = jnp.full(mb_scr.shape, -jnp.inf, _F32)

        NCB = S // CB
        CPR = 2048 // CB

        def ckv_chunk(t):
            b = t // NCB
            j = t % NCB
            return ckv_buf[b * 4 + j // CPR, pl.ds(_mult((j % CPR) * CB, CB), CB), :]

        def b_scores(t):
            b = t // NCB
            j = t % NCB
            s = _dot_nt(qab_scr[b], ckv_chunk(t))
            sb_scr[b, :, pl.ds(_mult(j * CB, CB), CB)] = s
            mb_scr[b] = jnp.maximum(mb_scr[b], fold(s, jnp.maximum))

        def b_scores_done():
            for b in range(B):
                m = jnp.max(mb_scr[b], axis=1, keepdims=True)
                mb_scr[b] = jnp.broadcast_to(m, (H, 128))
            lb_scr[...] = jnp.zeros_like(lb_scr)
            ctx_scr[...] = jnp.zeros_like(ctx_scr)

        def b_ctx(t):
            b = t // NCB
            j = t % NCB
            s = sb_scr[b, :, pl.ds(_mult(j * CB, CB), CB)]
            m = mb_scr[b]
            p = jnp.concatenate(
                [jnp.exp((s[:, u * 128:(u + 1) * 128] - m) * scale)
                 for u in range(CB // 128)], axis=1)
            lb_scr[b] += fold(p, jnp.add)
            ctx_scr[b] += _dot(p.astype(_BF16), ckv_chunk(t))

        def b_ctx_done():
            for b in range(B):
                ctx_scr[b] = ctx_scr[b] / jnp.sum(lb_scr[b], axis=1, keepdims=True)
            ob_scr[...] = jnp.zeros_like(ob_scr)

        def b_value(t):
            a, r, tiles = head_tiles(wuv_buf, t)
            rows = pl.ds(_mult(a * 8, 8), 8)
            cols = pl.ds(_mult(r * 128, 128), 128)
            lhs = jnp.concatenate(
                [ctx_scr[b, rows, cols] for b in range(B)], axis=0).astype(_BF16)
            ctxc_scr[a] += pick([_dot(lhs, w) for w in tiles])

        def b_out(t):
            a = t // 2
            k0 = (t % 2) * 4
            lhs = ctxc_scr[a].astype(_BF16)
            parts = [
                _dot(lhs, wob_buf[a, pl.ds(_mult((k0 + j) * D, D), D), :])
                for j in range(4)
            ]
            k = lax.broadcasted_iota(jnp.int32, (16, M), 0) % 8
            y = jnp.where(k == k0, parts[0], 0.0)
            for j in range(1, 4):
                y = jnp.where(k == k0 + j, parts[j], y)
            ob_scr[...] += y

        def b_done():
            for b in range(B):
                ob = jnp.sum(ob_scr[b * 8:(b + 1) * 8, :], axis=0, keepdims=True)
                out_ref[b:b + 1, M:2 * M] = ob.astype(out_ref.dtype)

        cp_xa.start()
        cp_xb.start()

        def prologue(it, carry):
            for c in range(P):
                ucp(0, 0, it * P + c).start(priority=_HI)
                ucp(0, 1, it * P + c).start(priority=_LO)
            return carry

        lax.fori_loop(0, BV, prologue, 0)

        def seg_loop(seg, lo, hi, extra=None):
            nxt = lo + BV >= UI

            def body(it, carry):
                for c in range(P):
                    ucp(seg, 1, it * P + c).wait()
                    if not nxt:
                        ucp(seg, 0, (it + BV) * P + c).start(priority=_HI)
                        ucp(seg, 1, (it + BV) * P + c).start(priority=_LO)
                    elif seg + 1 < NSEG:
                        ucp(seg + 1, 0, (it + BV - UI) * P + c).start(priority=_HI)
                        ucp(seg + 1, 1, (it + BV - UI) * P + c).start(priority=_LO)
                    else:
                        kcp(it + BV - UI, c).start(priority=_HI)
                        vcp(it + BV - UI, c).start(priority=_LO)
                    if c == 0 and extra is not None:
                        extra(it)
                return carry

            lax.fori_loop(lo, hi, body, 0)

        for seg in range(NSEG):
            if seg == 1:
                uwait_all(0)
                cp_xa.wait()
                cp_xb.wait()
                for k in range(4):
                    seg_loop(seg, k, k + 1, extra=lambda it, k=k: qa_task(k))
                seg_loop(seg, 4, UI - BV)
            else:
                seg_loop(seg, 0, UI - BV)
            seg_loop(seg, UI - BV, UI)
        for seg in range(1, NSEG):
            uwait_all(seg)

        reset_group()
        oa_scr[...] = jnp.zeros_like(oa_scr)

        def first_block(i, carry):
            kwait_all(i)
            for c in range(P):
                kcp(i + XK, c).start(priority=_HI)
            qk(i)
            return carry

        lax.fori_loop(0, G, first_block, 0)
        softmax_update()
        kwait_all(G)

        def end_of_piece(i):
            @pl.when(i % G == G - 1)
            def _():
                @pl.when(i % PPG == PPG - 1)
                def _():
                    finish_group(i // PPG)
                    reset_group()

                softmax_update()

        def main_loop(lo, hi, extra=None):
            def body(i, carry):
                def issue(c):
                    kcp(i + G + XK, c).start(priority=_HI)
                    vcp(i + BV, c).start(priority=_LO)

                vcp(i, 0).wait()
                issue(0)
                qk(i + G)
                if extra is not None:
                    extra(i - lo)
                for c in range(1, P):
                    vcp(i, c).wait()
                    issue(c)
                pv(i)
                kwait_all(i + G + 1)
                end_of_piece(i)
                return carry

            lax.fori_loop(lo, hi, body, 0)

        def tail_loop(lo, hi):
            def body(i, carry):
                for c in range(P):
                    vcp(i, c).wait()

                    @pl.when(i + BV < NP - G)
                    def _():
                        vcp(i + BV, c).start(priority=_LO)

                    @pl.when(jnp.logical_and(i + BV >= NP - G, i + BV < NP))
                    def _():
                        vcp_last(i + BV, c).start(priority=_LO)

                qk(i + G)
                pv(i)

                @pl.when(i + G + 1 < NP)
                def _():
                    kwait_all(i + G + 1)

                end_of_piece(i)
                return carry

            lax.fori_loop(lo, hi, body, 0)

        def last_block():
            g = NG - 1
            row = lax.broadcasted_iota(jnp.int32, (R, M), 0)
            rl = inv_l()
            y = oa_scr[B - 1]
            for u in range(G):
                i = NP - G + u
                for c in range(P):
                    vcp_last(i, c).wait()
                    if i + BV < NP:
                        vcp_last(i + BV, c).start(priority=_LO)
                slot = i % NV
                rowd = lax.broadcasted_iota(jnp.int32, (R, D), 0)
                o = None
                for e in range(HPP):
                    oe = functools.reduce(jnp.add, [
                        _dot(p_scr[:, kt * KP:(kt + 1) * KP], vbuf[slot, e * G + kt])
                        for kt in range(G)])
                    o = oe if o is None else jnp.where(rowd == u * HPP + e, oe, o)
                o = ((acc_scr[...] + o) * rl).astype(_BF16)
                for e in range(HPP):
                    r = u * HPP + e
                    yr = _dot(o, wo_buf[g % GPB, r * D:(r + 1) * D, :])
                    y = y + jnp.where(row == r, yr, 0.0)
            out_ref[B - 1:B, 0:M] = jnp.sum(y, axis=0, keepdims=True).astype(out_ref.dtype)

        b_init()
        pos = 0
        for n, task, done in [
            (16, b_query, None),
            (16, b_absorb, b_absorb_done),
            (B * NCB, b_scores, b_scores_done),
            (B * NCB, b_ctx, b_ctx_done),
            (16, b_value, None),
            (8, b_out, b_done),
        ]:
            main_loop(pos, pos + n, extra=task)
            pos += n
            if done is not None:
                done()
        tail0 = NP - G - XK
        assert XK >= BV
        assert pos <= tail0 and P % G == 0 and HPP * G == R and P == R
        main_loop(pos, tail0)
        for b in range(B - 1):
            oa = jnp.sum(oa_scr[b], axis=0, keepdims=True)
            out_ref[b:b + 1, 0:M] = oa.astype(out_ref.dtype)
        tail_loop(tail0, NP - G)
        last_block()

    scratch = [
        pltpu.VMEM((B, M), _BF16),
        pltpu.VMEM((B, M), _BF16),
        pltpu.VMEM((8, 64, HD), _BF16),
        pltpu.VMEM((4, 1024, M), _BF16),
        pltpu.VMEM((4, 4096, D), _BF16),
        pltpu.VMEM((4, 4096, D), _BF16),
        pltpu.VMEM((4, 4096, D), _BF16),
        pltpu.VMEM((4, 1024, M), _BF16),
        pltpu.VMEM((8, 2048, M), _BF16),
        pltpu.VMEM((NK, R, KP, D), _BF16),
        pltpu.VMEM((NV, R, KP, D), _BF16),
        pltpu.VMEM((NG, R, D), _F32),
        pltpu.VMEM((R, KB), _F32),
        pltpu.VMEM((R, KB), _BF16),
        pltpu.VMEM((R, D), _F32),
        pltpu.VMEM((R, D), _F32),
        pltpu.VMEM((R, D), _F32),
        pltpu.VMEM((B, R, M), _F32),
        pltpu.VMEM((16, M), _BF16),
        pltpu.VMEM((GPB, 16, D), _F32),
        pltpu.VMEM((B, H, M), _F32),
        pltpu.VMEM((B, H, M), _BF16),
        pltpu.VMEM((B, H, S), _F32),
        pltpu.VMEM((B, H, 128), _F32),
        pltpu.VMEM((B, H, 128), _F32),
        pltpu.VMEM((B, H, M), _F32),
        pltpu.VMEM((GPB, 16, D), _F32),
        pltpu.VMEM((16, M), _F32),
    ]

    def call(A_x, A_k_cache, A_v_cache, A_wq, A_wo, B_x, B_c_kv, B_w_q, B_w_uk,
             B_w_uv, B_w_o):
        any_spec = pl.BlockSpec(memory_space=pl.ANY)
        out = pl.pallas_call(
            kernel,
            out_shape=jax.ShapeDtypeStruct((B, 2 * M), _BF16),
            in_specs=[any_spec] * 11,
            out_specs=pl.BlockSpec(memory_space=pltpu.VMEM),
            scratch_shapes=scratch,
            compiler_params=pltpu.CompilerParams(
                vmem_limit_bytes=100 * 1024 * 1024,
                disable_bounds_checks=True),
        )(
            A_x.reshape(B, M),
            A_k_cache.reshape(NBH, S, D),
            A_v_cache.reshape(NBH, S, D),
            A_wq.reshape(8, 64, HD),
            A_wo.reshape(4, 1024, M),
            B_x.reshape(B, M),
            B_c_kv.reshape(8, 2048, M),
            B_w_q.reshape(4, 4096, D),
            B_w_uk.reshape(4, 4096, D),
            B_w_uv.reshape(4, 4096, D),
            B_w_o.reshape(4, 1024, M),
        )
        return out.reshape(B, 1, 2 * M)

    return call


@jax.jit
def pallas_concat_heads__gqa_block_cached__compressed_kv_cla__decode_kernel(
    A_x: jax.Array,
    A_k_cache: jax.Array,
    A_v_cache: jax.Array,
    A_wq: jax.Array,
    A_wo: jax.Array,
    B_x: jax.Array,
    B_c_kv: jax.Array,
    B_w_q: jax.Array,
    B_w_uk: jax.Array,
    B_w_uv: jax.Array,
    B_w_o: jax.Array,
):
    B, H, S, D = A_k_cache.shape
    M = A_x.shape[-1]
    assert A_x.shape == (B, 1, M) and B_x.shape == (B, 1, M)
    assert A_wq.shape == (M, H * D) and B_c_kv.shape == (B, S, M)
    assert B_w_q.shape == (M, H, D) and B_w_o.shape == (H, D, M)
    return _build(B, H, S, D, M)(A_x, A_k_cache, A_v_cache, A_wq, A_wo, B_x,
                                 B_c_kv, B_w_q, B_w_uk, B_w_uv, B_w_o)
```

```python
import functools

import jax
import jax.numpy as jnp
from jax import lax
import jax.experimental.pallas as pl
import jax.experimental.pallas.tpu as pltpu

_NT = (((1,), (1,)), ((), ()))
_BF16 = jnp.bfloat16
_F32 = jnp.float32
_HI, _LO = 0, 1


def _dot(a, b):
    return jnp.dot(a, b, preferred_element_type=_F32)


def _dot_nt(a, b):
    return lax.dot_general(a, b, _NT, preferred_element_type=_F32)


def _mult(x, m):
    return x if isinstance(x, int) else pl.multiple_of(x, m)


def _build(B, H, S, D, M, XK=8, BV=6, XH=2, KB=512, CB=256):
    R = 8
    C = 16
    KP = 128
    P = KP // C
    G = KB // KP
    PPG = S // KP
    NBH = B * H
    GPB = H // R
    NG = NBH // R
    NP = NG * PPG
    NK = XK + 2
    NV = BV + 2
    HD = H * D
    scale = float(D) ** -0.5
    UD = 128
    UI = UD // P
    assert M == 512 and D == 128 and HD == 4096 and B == 2

    def kernel(xa_hbm, k_hbm, v_hbm, wq_hbm, wo_hbm, xb_hbm, ckv_hbm, wqb_hbm,
               wuk_hbm, wuv_hbm, wob_hbm, out_ref,
               xa_buf, xb_buf, wq_buf, wo_buf, wqb_buf, wuk_buf, wuv_buf, wob_buf,
               ckv_buf, kbuf, vbuf, q_scr, s_scr, p_scr, m_scr, l_scr, acc_scr,
               oa_scr, xb16_scr, qb_scr, qabs_scr, qab_scr, sb_scr, mb_scr, lb_scr, ctx_scr,
               ctxc_scr, ob_scr):
        pl.run_scoped(
            functools.partial(
                body_fn, xa_hbm, k_hbm, v_hbm, wq_hbm, wo_hbm, xb_hbm, ckv_hbm,
                wqb_hbm, wuk_hbm, wuv_hbm, wob_hbm, out_ref,
                xa_buf, xb_buf, wq_buf, wo_buf, wqb_buf, wuk_buf, wuv_buf, wob_buf,
                ckv_buf, kbuf, vbuf, q_scr, s_scr, p_scr, m_scr, l_scr, acc_scr,
                oa_scr, xb16_scr, qb_scr, qabs_scr, qab_scr, sb_scr, mb_scr, lb_scr,
                ctx_scr, ctxc_scr, ob_scr),
            pltpu.SemaphoreType.DMA((2,)),
            pltpu.SemaphoreType.DMA((11,)),
            pltpu.SemaphoreType.DMA((NK,)),
            pltpu.SemaphoreType.DMA((NV,)),
        )

    def body_fn(xa_hbm, k_hbm, v_hbm, wq_hbm, wo_hbm, xb_hbm, ckv_hbm, wqb_hbm,
                wuk_hbm, wuv_hbm, wob_hbm, out_ref,
                xa_buf, xb_buf, wq_buf, wo_buf, wqb_buf, wuk_buf, wuv_buf, wob_buf,
                ckv_buf, kbuf, vbuf, q_scr, s_scr, p_scr, m_scr, l_scr, acc_scr,
                oa_scr, xb16_scr, qb_scr, qabs_scr, qab_scr, sb_scr, mb_scr, lb_scr,
                ctx_scr, ctxc_scr, ob_scr, semx, semu, semk, semv):
        cp_xa = pltpu.make_async_copy(xa_hbm, xa_buf, semx.at[0])
        cp_xb = pltpu.make_async_copy(xb_hbm, xb_buf, semx.at[1])

        def unit_wq(j):
            idx = (slice(None), pl.ds(_mult((j // 16) * 8, 8), 8),
                   pl.ds(_mult((j % 16) * 256, 256), 256))
            return wq_hbm.at[idx], wq_buf.at[idx]

        def unit_rows(hbm, buf):
            def f(j):
                idx = (slice(None), pl.ds(_mult(j * 32, 32), 32), slice(None))
                return hbm.at[idx], buf.at[idx]
            return f

        def unit_wide(hbm, buf):
            def f(j):
                idx = (slice(None), pl.ds(_mult(j * 8, 8), 8), slice(None))
                return hbm.at[idx], buf.at[idx]
            return f

        def unit_ckv(u):
            def f(j):
                idx = (slice(None), pl.ds(_mult(u * 512 + (j // 2) * 8, 8), 8),
                       pl.ds(_mult((j % 2) * 256, 256), 256))
                return ckv_hbm.at[idx], ckv_buf.at[idx]
            return f

        def view_wq(p0, p1):
            assert p0 % 2 == 0 and p1 % 2 == 0
            return wq_buf.at[:, pl.ds(p0 * 4, (p1 - p0) * 4), :]

        def view_rows(buf):
            return lambda p0, p1: buf.at[:, pl.ds(p0 * P * 32, (p1 - p0) * P * 32), :]

        def view_wide(buf):
            return lambda p0, p1: buf.at[:, pl.ds(p0 * P * 8, (p1 - p0) * P * 8), :]

        def view_ckv(u):
            return lambda p0, p1: ckv_buf.at[
                :, pl.ds(u * 512 + p0 * P * 4, (p1 - p0) * P * 4), :]

        def rows_unit(hbm, buf):
            return unit_rows(hbm, buf), view_rows(buf)

        def wide_unit(hbm, buf):
            return unit_wide(hbm, buf), view_wide(buf)

        units = {
            "wq": (unit_wq, view_wq),
            "wqb": rows_unit(wqb_hbm, wqb_buf),
            "wuk": rows_unit(wuk_hbm, wuk_buf),
            "wuv": rows_unit(wuv_hbm, wuv_buf),
            "wo": wide_unit(wo_hbm, wo_buf),
            "wob": wide_unit(wob_hbm, wob_buf),
        }
        for u in range(4):
            units["c%d" % u] = (unit_ckv(u), view_ckv(u))
        shift = (G + XK - XH) // 2
        assert 2 * shift == G + XK - XH and 0 <= shift < UI
        hi_runs = [("wq", 0, UI), ("c0", 0, UI), ("c1", 0, UI), ("c2", 0, UI),
                   ("c3", 0, UI - shift)]
        lo_runs = [("wqb", 0, UI), ("wuk", 0, UI), ("wuv", 0, UI), ("wo", 0, UI),
                   ("wob", 0, UI), ("c3", UI - shift, UI)]
        lo_runs = [r for r in lo_runs if r[2] > r[1]]
        hi_seq = [(n, q) for n, (_, p0, p1) in enumerate(hi_runs) for q in range(p0, p1)]
        lo_seq = [(n, q) for n, (_, p0, p1) in enumerate(lo_runs) for q in range(p0, p1)]
        NHI, NLO = len(hi_seq), len(lo_seq)

        def ucp(side, n, q, c):
            name = (hi_runs, lo_runs)[side][n][0]
            src, dst = units[name][0](q * P + c)
            sem = semu.at[n] if side == 0 else semu.at[len(hi_runs) + n]
            return pltpu.make_async_copy(src, dst, sem)

        def hi_run_wait(n):
            name, p0, p1 = hi_runs[n]
            ref = units[name][1](p0, p1)
            pltpu.make_async_copy(ref, ref, semu.at[n]).wait()

        def kv_src(hbm, i, c):
            g = i // PPG
            j = i % PPG
            return hbm.at[g // 2, :, g % 2, pl.ds(_mult(j * KP + c * C, C), C), :]

        def kcp(i, c):
            slot = i % NK
            return pltpu.make_async_copy(
                kv_src(k_hbm, i, c), kbuf.at[slot, :, pl.ds(c * C, C), :],
                semk.at[slot])

        def vcp(i, c):
            slot = i % NV
            return pltpu.make_async_copy(
                kv_src(v_hbm, i, c), vbuf.at[slot, :, pl.ds(c * C, C), :],
                semv.at[slot])

        HPP = R // G

        def vcp_last(i, c):
            u = i - (NP - G)
            slot = i % NV
            r = u * HPP + c // G
            key0 = S - KB + (c % G) * KP
            return pltpu.make_async_copy(
                v_hbm.at[(NG - 1) // 2, r, (NG - 1) % 2, pl.ds(key0, KP), :],
                vbuf.at[slot, c], semv.at[slot])

        def kwait_all(i):
            slot = i % NK
            pltpu.make_async_copy(kbuf.at[slot], kbuf.at[slot], semk.at[slot]).wait()

        def x16(buf):
            x = buf[...].astype(_F32)
            row = lax.broadcasted_iota(jnp.int32, (16, M), 0)
            z = jnp.where(row < 8, jnp.broadcast_to(x[0:1, :], (16, M)),
                          jnp.broadcast_to(x[1:2, :], (16, M)))
            return z.astype(_BF16)

        def pick(parts, k0=0):
            shape = parts[0].shape
            k = lax.broadcasted_iota(jnp.int32, shape, 0) % 8
            res = parts[0]
            for j in range(1, len(parts)):
                res = jnp.where(k == k0 + j, parts[j], res)
            return res

        def head_tiles(w_buf, t):
            a = t // 4
            r = t % 4
            n32 = M // 4 * H // 2
            sub = w_buf.bitcast(jnp.uint32).at[
                r, pl.ds(pl.multiple_of(4 * a, 4), n32 - 12), :]
            tiles = []
            for u in range(4):
                w = sub[pl.ds(u, 128, stride=H // 2), :]
                even = pltpu.bitcast(w << 16, _F32).astype(_BF16)
                odd = pltpu.bitcast(w & jnp.uint32(0xFFFF0000), _F32).astype(_BF16)
                tiles += [even, odd]
            return a, r, tiles

        def fold(x, op):
            r = x[:, 0:128]
            for t in range(1, x.shape[1] // 128):
                r = op(r, x[:, t * 128:(t + 1) * 128])
            return r

        def qa_task(k):
            w = wq_buf[:, :, k * 1024:(k + 1) * 1024].reshape(M, 1024)
            qa = _dot(x16(xa_buf), w)
            r0 = 4 * (k % 2)
            for par in range(2):
                cols = [qa[:, (2 * j + par) * D:(2 * j + par + 1) * D] for j in range(4)]
                q = pick(cols, r0)
                for b in range(B):
                    g = b * GPB + (k // 2) * 2 + par
                    q_scr[g, r0:r0 + 4, :] = q[b * R + r0:b * R + r0 + 4, :]

        def wo_head(g, r):
            half = (g // 2) % 2
            off = ((2 * r) % 8 + g % 2) * D
            return wo_buf[half * 2 + r // 4, pl.ds(_mult(off, D), D), :]

        def qk(i):
            g = i // PPG
            j = i % G
            q = q_scr[g].astype(_BF16)
            slot = i % NK
            s = pick([_dot_nt(q, kbuf[slot, r]) for r in range(R)])
            s_scr[:, pl.ds(_mult(j * KP, KP), KP)] = s

        def softmax_update():
            s = [s_scr[:, t * 128:(t + 1) * 128] for t in range(KB // 128)]
            mx = functools.reduce(jnp.maximum, s)
            m_old = m_scr[...]
            m_new = jnp.maximum(m_old, jnp.max(mx, axis=1, keepdims=True))
            alpha = jnp.exp((m_old - m_new) * scale)
            p = [jnp.exp((st - m_new) * scale) for st in s]
            l_scr[...] = l_scr[...] * alpha + functools.reduce(jnp.add, p)
            m_scr[...] = m_new
            acc_scr[...] = acc_scr[...] * alpha
            for t in range(KB // 128):
                p_scr[:, t * 128:(t + 1) * 128] = p[t].astype(_BF16)

        def inv_l():
            return 1.0 / jnp.sum(l_scr[...], axis=1, keepdims=True)

        def pv(i):
            j = i % G
            slot = i % NV
            p = p_scr[:, pl.ds(_mult(j * KP, KP), KP)]
            acc_scr[...] += pick([_dot(p, vbuf[slot, r]) for r in range(R)])

        def reset_group():
            acc_scr[...] = jnp.zeros_like(acc_scr)
            l_scr[...] = jnp.zeros_like(l_scr)
            m_scr[...] = jnp.full(m_scr.shape, -jnp.inf, _F32)

        def finish_group(g):
            o = (acc_scr[...] * inv_l()).astype(_BF16)
            oa_scr[g // GPB] += pick([_dot(o, wo_head(g, r)) for r in range(R)])

        def b_init():
            xb16_scr[...] = x16(xb_buf)
            qb_scr[...] = jnp.zeros_like(qb_scr)
            ctxc_scr[...] = jnp.zeros_like(ctxc_scr)

        def b_query(t):
            a, r, tiles = head_tiles(wqb_buf, t)
            x = xb16_scr[:, pl.ds(_mult(r * 128, 128), 128)]
            qb_scr[a] += pick([_dot(x, w) for w in tiles])

        def b_absorb(t):
            a, r, tiles = head_tiles(wuk_buf, t)
            q = qb_scr[a].astype(_BF16)
            qabs = pick([_dot_nt(q, w) for w in tiles])
            for b in range(B):
                qabs_scr[b, pl.ds(_mult(a * 8, 8), 8),
                         pl.ds(_mult(r * 128, 128), 128)] = qabs[b * 8:(b + 1) * 8, :]

        def b_absorb_done():
            qab_scr[...] = qabs_scr[...].astype(_BF16)
            mb_scr[...] = jnp.full(mb_scr.shape, -jnp.inf, _F32)

        NCB = S // CB
        CPR = 2048 // CB

        def ckv_chunk(t):
            b = t // NCB
            j = t % NCB
            return ckv_buf[b * 4 + j // CPR, pl.ds(_mult((j % CPR) * CB, CB), CB), :]

        def b_scores(t):
            b = t // NCB
            j = t % NCB
            s = _dot_nt(qab_scr[b], ckv_chunk(t))
            sb_scr[b, :, pl.ds(_mult(j * CB, CB), CB)] = s
            mb_scr[b] = jnp.maximum(mb_scr[b], fold(s, jnp.maximum))

        def b_scores_done():
            for b in range(B):
                m = jnp.max(mb_scr[b], axis=1, keepdims=True)
                mb_scr[b] = jnp.broadcast_to(m, (H, 128))
            lb_scr[...] = jnp.zeros_like(lb_scr)
            ctx_scr[...] = jnp.zeros_like(ctx_scr)

        def b_ctx(t):
            b = t // NCB
            j = t % NCB
            s = sb_scr[b, :, pl.ds(_mult(j * CB, CB), CB)]
            m = mb_scr[b]
            p = jnp.concatenate(
                [jnp.exp((s[:, u * 128:(u + 1) * 128] - m) * scale)
                 for u in range(CB // 128)], axis=1)
            lb_scr[b] += fold(p, jnp.add)
            ctx_scr[b] += _dot(p.astype(_BF16), ckv_chunk(t))

        def b_ctx_done():
            for b in range(B):
                ctx_scr[b] = ctx_scr[b] / jnp.sum(lb_scr[b], axis=1, keepdims=True)
            ob_scr[...] = jnp.zeros_like(ob_scr)

        def b_value(t):
            a, r, tiles = head_tiles(wuv_buf, t)
            rows = pl.ds(_mult(a * 8, 8), 8)
            cols = pl.ds(_mult(r * 128, 128), 128)
            lhs = jnp.concatenate(
                [ctx_scr[b, rows, cols] for b in range(B)], axis=0).astype(_BF16)
            ctxc_scr[a] += pick([_dot(lhs, w) for w in tiles])

        def b_out(t):
            a = t // 2
            k0 = (t % 2) * 4
            lhs = ctxc_scr[a].astype(_BF16)
            parts = [
                _dot(lhs, wob_buf[a, pl.ds(_mult((k0 + j) * D, D), D), :])
                for j in range(4)
            ]
            k = lax.broadcasted_iota(jnp.int32, (16, M), 0) % 8
            y = jnp.where(k == k0, parts[0], 0.0)
            for j in range(1, 4):
                y = jnp.where(k == k0 + j, parts[j], y)
            ob_scr[...] += y

        def b_done():
            for b in range(B):
                ob = jnp.sum(ob_scr[b * 8:(b + 1) * 8, :], axis=0, keepdims=True)
                out_ref[b:b + 1, M:2 * M] = ob.astype(out_ref.dtype)

        cp_xa.start()
        cp_xb.start()

        def prologue(it, carry):
            for c in range(P):
                ucp(1, 0, it, c).start(priority=_LO)
            return carry

        def prologue_hi(it, carry):
            for c in range(P):
                ucp(0, 0, it, c).start(priority=_HI)
            return carry

        lax.fori_loop(0, XH, prologue_hi, 0)
        lax.fori_loop(0, BV, prologue, 0)

        def first_block(t):
            i = t - (NLO - G)
            kwait_all(i)
            qk(i)

        QA0 = UI + 2

        def plan(t):
            wn, wq_ = lo_seq[t]
            h = hi_seq[t + XH] if t + XH < NHI else (-1, t + XH - NHI)
            l = lo_seq[t + BV] if t + BV < NLO else (-1, t + BV - NLO)
            if QA0 <= t < QA0 + 4:
                ex = ("qa", t - QA0)
            elif t >= NLO - G:
                ex = ("first",)
            else:
                ex = None
            return (wn, h[0], l[0], ex), (wq_ - t, h[1] - t, l[1] - t)

        def phase1_loop(t0, t1):
            (wn, hn, ln, ex), (wo_, ho, lo_) = plan(t0)

            def body(t, carry):
                for c in range(P):
                    ucp(1, wn, t + wo_, c).wait()
                    if hn >= 0:
                        ucp(0, hn, t + ho, c).start(priority=_HI)
                    else:
                        kcp(t + ho, c).start(priority=_HI)
                    if ln >= 0:
                        ucp(1, ln, t + lo_, c).start(priority=_LO)
                    else:
                        vcp(t + lo_, c).start(priority=_LO)
                    if c == 0 and ex is not None:
                        if ex[0] == "qa":
                            qa_task(ex[1])
                        else:
                            first_block(t)
                return carry

            lax.fori_loop(t0, t1, body, 0)

        reset_group()
        oa_scr[...] = jnp.zeros_like(oa_scr)
        t0 = 0
        for t in range(1, NLO + 1):
            if t == NLO or plan(t) != plan(t0):
                if t0 == QA0:
                    hi_run_wait(0)
                    cp_xa.wait()
                    cp_xb.wait()
                phase1_loop(t0, t)
                t0 = t
        for n in range(1, len(hi_runs)):
            hi_run_wait(n)
        softmax_update()
        kwait_all(G)

        def end_of_piece(i):
            @pl.when(i % G == G - 1)
            def _():
                @pl.when(i % PPG == PPG - 1)
                def _():
                    finish_group(i // PPG)
                    reset_group()

                softmax_update()

        def main_loop(lo, hi, extra=None):
            def body(i, carry):
                def issue(c):
                    kcp(i + G + XK, c).start(priority=_HI)
                    vcp(i + BV, c).start(priority=_LO)

                vcp(i, 0).wait()
                issue(0)
                qk(i + G)
                if extra is not None:
                    extra(i - lo)
                for c in range(1, P):
                    vcp(i, c).wait()
                    issue(c)
                pv(i)
                kwait_all(i + G + 1)
                end_of_piece(i)
                return carry

            lax.fori_loop(lo, hi, body, 0)

        def tail_loop(lo, hi):
            def body(i, carry):
                for c in range(P):
                    vcp(i, c).wait()

                    @pl.when(i + BV < NP - G)
                    def _():
                        vcp(i + BV, c).start(priority=_LO)

                    @pl.when(jnp.logical_and(i + BV >= NP - G, i + BV < NP))
                    def _():
                        vcp_last(i + BV, c).start(priority=_LO)

                qk(i + G)
                pv(i)

                @pl.when(i + G + 1 < NP)
                def _():
                    kwait_all(i + G + 1)

                end_of_piece(i)
                return carry

            lax.fori_loop(lo, hi, body, 0)

        def last_block():
            g = NG - 1
            row = lax.broadcasted_iota(jnp.int32, (R, M), 0)
            rl = inv_l()
            y = oa_scr[B - 1]
            for u in range(G):
                i = NP - G + u
                for c in range(P):
                    vcp_last(i, c).wait()
                    if i + BV < NP:
                        vcp_last(i + BV, c).start(priority=_LO)
                slot = i % NV
                rowd = lax.broadcasted_iota(jnp.int32, (R, D), 0)
                o = None
                for e in range(HPP):
                    oe = functools.reduce(jnp.add, [
                        _dot(p_scr[:, kt * KP:(kt + 1) * KP], vbuf[slot, e * G + kt])
                        for kt in range(G)])
                    o = oe if o is None else jnp.where(rowd == u * HPP + e, oe, o)
                o = ((acc_scr[...] + o) * rl).astype(_BF16)
                for e in range(HPP):
                    r = u * HPP + e
                    yr = _dot(o, wo_head(g, r))
                    y = y + jnp.where(row == r, yr, 0.0)
            out_ref[B - 1:B, 0:M] = jnp.sum(y, axis=0, keepdims=True).astype(out_ref.dtype)

        b_init()
        pos = 0
        for n, task, done in [
            (16, b_query, None),
            (16, b_absorb, b_absorb_done),
            (B * NCB, b_scores, b_scores_done),
            (B * NCB, b_ctx, b_ctx_done),
            (16, b_value, None),
            (8, b_out, b_done),
        ]:
            main_loop(pos, pos + n, extra=task)
            pos += n
            if done is not None:
                done()
        tail0 = NP - G - XK
        assert XK >= BV - G
        assert pos <= tail0 and P % G == 0 and HPP * G == R and P == R
        main_loop(pos, tail0)
        for b in range(B - 1):
            oa = jnp.sum(oa_scr[b], axis=0, keepdims=True)
            out_ref[b:b + 1, 0:M] = oa.astype(out_ref.dtype)
        tail_loop(tail0, NP - G)
        last_block()

    scratch = [
        pltpu.VMEM((B, M), _BF16),
        pltpu.VMEM((B, M), _BF16),
        pltpu.VMEM((8, 64, HD), _BF16),
        pltpu.VMEM((4, 1024, M), _BF16),
        pltpu.VMEM((4, 4096, D), _BF16),
        pltpu.VMEM((4, 4096, D), _BF16),
        pltpu.VMEM((4, 4096, D), _BF16),
        pltpu.VMEM((4, 1024, M), _BF16),
        pltpu.VMEM((8, 2048, M), _BF16),
        pltpu.VMEM((NK, R, KP, D), _BF16),
        pltpu.VMEM((NV, R, KP, D), _BF16),
        pltpu.VMEM((NG, R, D), _F32),
        pltpu.VMEM((R, KB), _F32),
        pltpu.VMEM((R, KB), _BF16),
        pltpu.VMEM((R, D), _F32),
        pltpu.VMEM((R, D), _F32),
        pltpu.VMEM((R, D), _F32),
        pltpu.VMEM((B, R, M), _F32),
        pltpu.VMEM((16, M), _BF16),
        pltpu.VMEM((GPB, 16, D), _F32),
        pltpu.VMEM((B, H, M), _F32),
        pltpu.VMEM((B, H, M), _BF16),
        pltpu.VMEM((B, H, S), _F32),
        pltpu.VMEM((B, H, 128), _F32),
        pltpu.VMEM((B, H, 128), _F32),
        pltpu.VMEM((B, H, M), _F32),
        pltpu.VMEM((GPB, 16, D), _F32),
        pltpu.VMEM((16, M), _F32),
    ]

    def call(A_x, A_k_cache, A_v_cache, A_wq, A_wo, B_x, B_c_kv, B_w_q, B_w_uk,
             B_w_uv, B_w_o):
        any_spec = pl.BlockSpec(memory_space=pl.ANY)
        out = pl.pallas_call(
            kernel,
            out_shape=jax.ShapeDtypeStruct((B, 2 * M), _BF16),
            in_specs=[any_spec] * 11,
            out_specs=pl.BlockSpec(memory_space=pltpu.VMEM),
            scratch_shapes=scratch,
            compiler_params=pltpu.CompilerParams(
                vmem_limit_bytes=100 * 1024 * 1024,
                disable_bounds_checks=True),
        )(
            A_x.reshape(B, M),
            A_k_cache.reshape(B * 2, R, 2, S, D),
            A_v_cache.reshape(B * 2, R, 2, S, D),
            A_wq.reshape(8, 64, HD),
            A_wo.reshape(4, 1024, M),
            B_x.reshape(B, M),
            B_c_kv.reshape(8, 2048, M),
            B_w_q.reshape(4, 4096, D),
            B_w_uk.reshape(4, 4096, D),
            B_w_uv.reshape(4, 4096, D),
            B_w_o.reshape(4, 1024, M),
        )
        return out.reshape(B, 1, 2 * M)

    return call


@jax.jit
def pallas_concat_heads__gqa_block_cached__compressed_kv_cla__decode_kernel(
    A_x: jax.Array,
    A_k_cache: jax.Array,
    A_v_cache: jax.Array,
    A_wq: jax.Array,
    A_wo: jax.Array,
    B_x: jax.Array,
    B_c_kv: jax.Array,
    B_w_q: jax.Array,
    B_w_uk: jax.Array,
    B_w_uv: jax.Array,
    B_w_o: jax.Array,
):
    B, H, S, D = A_k_cache.shape
    M = A_x.shape[-1]
    assert A_x.shape == (B, 1, M) and B_x.shape == (B, 1, M)
    assert A_wq.shape == (M, H * D) and B_c_kv.shape == (B, S, M)
    assert B_w_q.shape == (M, H, D) and B_w_o.shape == (H, D, M)
    return _build(B, H, S, D, M)(A_x, A_k_cache, A_v_cache, A_wq, A_wo, B_x,
                                 B_c_kv, B_w_q, B_w_uk, B_w_uv, B_w_o)
```

```python
import functools

import jax
import jax.numpy as jnp
from jax import lax
import jax.experimental.pallas as pl
import jax.experimental.pallas.tpu as pltpu

_NT = (((1,), (1,)), ((), ()))
_BF16 = jnp.bfloat16
_F32 = jnp.float32
_HI, _LO = 0, 1


def _dot(a, b):
    return jnp.dot(a, b, preferred_element_type=_F32)


def _dot_nt(a, b):
    return lax.dot_general(a, b, _NT, preferred_element_type=_F32)


def _mult(x, m):
    return x if isinstance(x, int) else pl.multiple_of(x, m)


def _build(B, H, S, D, M, XK=8, BV=6, XH=2, KB=512, CB=256):
    R = 8
    C = 16
    KP = 128
    P = KP // C
    G = KB // KP
    PPG = S // KP
    NBH = B * H
    GPB = H // R
    NG = NBH // R
    NP = NG * PPG
    NK = XK + 2
    NV = BV + 2
    HD = H * D
    scale = float(D) ** -0.5
    UD = 128
    UI = UD // P
    assert M == 512 and D == 128 and HD == 4096 and B == 2

    def kernel(xa_hbm, k_hbm, v_hbm, wq_hbm, wo_hbm, xb_hbm, ckv_hbm, wqb_hbm,
               wuk_hbm, wuv_hbm, wob_hbm, out_ref,
               xa_buf, xb_buf, wq_buf, wo_buf, wqb_buf, wuk_buf, wuv_buf, wob_buf,
               ckv_buf, kbuf, vbuf, q_scr, s_scr, p_scr, m_scr, l_scr, acc_scr,
               oa_scr, xb16_scr, qb_scr, qabs_scr, qab_scr, sb_scr, mb_scr, lb_scr, ctx_scr,
               ctxc_scr, ob_scr):
        pl.run_scoped(
            functools.partial(
                body_fn, xa_hbm, k_hbm, v_hbm, wq_hbm, wo_hbm, xb_hbm, ckv_hbm,
                wqb_hbm, wuk_hbm, wuv_hbm, wob_hbm, out_ref,
                xa_buf, xb_buf, wq_buf, wo_buf, wqb_buf, wuk_buf, wuv_buf, wob_buf,
                ckv_buf, kbuf, vbuf, q_scr, s_scr, p_scr, m_scr, l_scr, acc_scr,
                oa_scr, xb16_scr, qb_scr, qabs_scr, qab_scr, sb_scr, mb_scr, lb_scr,
                ctx_scr, ctxc_scr, ob_scr),
            pltpu.SemaphoreType.DMA((2,)),
            pltpu.SemaphoreType.DMA((11,)),
            pltpu.SemaphoreType.DMA((NK,)),
            pltpu.SemaphoreType.DMA((NV,)),
        )

    def body_fn(xa_hbm, k_hbm, v_hbm, wq_hbm, wo_hbm, xb_hbm, ckv_hbm, wqb_hbm,
                wuk_hbm, wuv_hbm, wob_hbm, out_ref,
                xa_buf, xb_buf, wq_buf, wo_buf, wqb_buf, wuk_buf, wuv_buf, wob_buf,
                ckv_buf, kbuf, vbuf, q_scr, s_scr, p_scr, m_scr, l_scr, acc_scr,
                oa_scr, xb16_scr, qb_scr, qabs_scr, qab_scr, sb_scr, mb_scr, lb_scr,
                ctx_scr, ctxc_scr, ob_scr, semx, semu, semk, semv):
        cp_xa = pltpu.make_async_copy(xa_hbm, xa_buf, semx.at[0])
        cp_xb = pltpu.make_async_copy(xb_hbm, xb_buf, semx.at[1])

        def unit_wq(j):
            idx = (slice(None), pl.ds(_mult((j // 16) * 8, 8), 8),
                   pl.ds(_mult((j % 16) * 256, 256), 256))
            return wq_hbm.at[idx], wq_buf.at[idx]

        def unit_rows(hbm, buf):
            def f(j):
                idx = (slice(None), pl.ds(_mult(j * 32, 32), 32), slice(None))
                return hbm.at[idx], buf.at[idx]
            return f

        def unit_wide(hbm, buf):
            def f(j):
                idx = (slice(None), pl.ds(_mult(j * 8, 8), 8), slice(None))
                return hbm.at[idx], buf.at[idx]
            return f

        def unit_ckv(u):
            def f(j):
                idx = (pl.ds((u // 2) * 8, 8),
                       pl.ds(_mult((u % 2) * 512 + (j // 2) * 8, 8), 8),
                       pl.ds(_mult((j % 2) * 256, 256), 256))
                return ckv_hbm.at[idx], ckv_buf.at[idx]
            return f

        def view_wq(p0, p1):
            assert p0 % 2 == 0 and p1 % 2 == 0
            return wq_buf.at[:, pl.ds(p0 * 4, (p1 - p0) * 4), :]

        def view_rows(buf):
            return lambda p0, p1: buf.at[:, pl.ds(p0 * P * 32, (p1 - p0) * P * 32), :]

        def view_wide(buf):
            return lambda p0, p1: buf.at[:, pl.ds(p0 * P * 8, (p1 - p0) * P * 8), :]

        def view_ckv(u):
            return lambda p0, p1: ckv_buf.at[
                pl.ds((u // 2) * 8, 8),
                pl.ds((u % 2) * 512 + p0 * P * 4, (p1 - p0) * P * 4), :]

        def rows_unit(hbm, buf):
            return unit_rows(hbm, buf), view_rows(buf)

        def wide_unit(hbm, buf):
            return unit_wide(hbm, buf), view_wide(buf)

        units = {
            "wq": (unit_wq, view_wq),
            "wqb": rows_unit(wqb_hbm, wqb_buf),
            "wuk": rows_unit(wuk_hbm, wuk_buf),
            "wuv": rows_unit(wuv_hbm, wuv_buf),
            "wo": wide_unit(wo_hbm, wo_buf),
            "wob": wide_unit(wob_hbm, wob_buf),
        }
        for u in range(4):
            units["c%d" % u] = (unit_ckv(u), view_ckv(u))
        shift = (G + XK - XH) // 2
        assert 2 * shift == G + XK - XH and 0 <= shift < UI
        hi_runs = [("wq", 0, UI), ("c0", 0, UI), ("c1", 0, UI), ("c2", 0, UI),
                   ("c3", 0, UI - shift)]
        lo_runs = [("wqb", 0, UI), ("wuk", 0, UI), ("wuv", 0, UI), ("wo", 0, UI),
                   ("wob", 0, UI), ("c3", UI - shift, UI)]
        lo_runs = [r for r in lo_runs if r[2] > r[1]]
        hi_seq = [(n, q) for n, (_, p0, p1) in enumerate(hi_runs) for q in range(p0, p1)]
        lo_seq = [(n, q) for n, (_, p0, p1) in enumerate(lo_runs) for q in range(p0, p1)]
        NHI, NLO = len(hi_seq), len(lo_seq)

        def ucp(side, n, q, c):
            name = (hi_runs, lo_runs)[side][n][0]
            src, dst = units[name][0](q * P + c)
            sem = semu.at[n] if side == 0 else semu.at[len(hi_runs) + n]
            return pltpu.make_async_copy(src, dst, sem)

        def hi_run_wait(n):
            name, p0, p1 = hi_runs[n]
            ref = units[name][1](p0, p1)
            pltpu.make_async_copy(ref, ref, semu.at[n]).wait()

        def kv_src(hbm, i, c):
            g = i // PPG
            j = i % PPG
            return hbm.at[g // 2, :, g % 2, pl.ds(_mult(j * KP + c * C, C), C), :]

        def kcp(i, c):
            slot = i % NK
            return pltpu.make_async_copy(
                kv_src(k_hbm, i, c), kbuf.at[slot, :, pl.ds(c * C, C), :],
                semk.at[slot])

        def vcp(i, c):
            slot = i % NV
            return pltpu.make_async_copy(
                kv_src(v_hbm, i, c), vbuf.at[slot, :, pl.ds(c * C, C), :],
                semv.at[slot])

        HPP = R // G

        def vcp_last(i, c):
            u = i - (NP - G)
            slot = i % NV
            r = u * HPP + c // G
            key0 = S - KB + (c % G) * KP
            return pltpu.make_async_copy(
                v_hbm.at[(NG - 1) // 2, r, (NG - 1) % 2, pl.ds(key0, KP), :],
                vbuf.at[slot, c], semv.at[slot])

        def kwait_all(i):
            slot = i % NK
            pltpu.make_async_copy(kbuf.at[slot], kbuf.at[slot], semk.at[slot]).wait()

        def x16(buf):
            x = buf[...].astype(_F32)
            row = lax.broadcasted_iota(jnp.int32, (16, M), 0)
            z = jnp.where(row < 8, jnp.broadcast_to(x[0:1, :], (16, M)),
                          jnp.broadcast_to(x[1:2, :], (16, M)))
            return z.astype(_BF16)

        def pick(parts, k0=0):
            shape = parts[0].shape
            k = lax.broadcasted_iota(jnp.int32, shape, 0) % 8
            res = parts[0]
            for j in range(1, len(parts)):
                res = jnp.where(k == k0 + j, parts[j], res)
            return res

        def head_tiles(w_buf, t):
            a = t // 4
            r = t % 4
            n32 = M // 4 * H // 2
            sub = w_buf.bitcast(jnp.uint32).at[
                r, pl.ds(pl.multiple_of(4 * a, 4), n32 - 12), :]
            tiles = []
            for u in range(4):
                w = sub[pl.ds(u, 128, stride=H // 2), :]
                even = pltpu.bitcast(w << 16, _F32).astype(_BF16)
                odd = pltpu.bitcast(w & jnp.uint32(0xFFFF0000), _F32).astype(_BF16)
                tiles += [even, odd]
            return a, r, tiles

        def fold(x, op):
            r = x[:, 0:128]
            for t in range(1, x.shape[1] // 128):
                r = op(r, x[:, t * 128:(t + 1) * 128])
            return r

        def qa_task(k):
            w = wq_buf[:, :, k * 1024:(k + 1) * 1024].reshape(M, 1024)
            qa = _dot(x16(xa_buf), w)
            r0 = 4 * (k % 2)
            for par in range(2):
                cols = [qa[:, (2 * j + par) * D:(2 * j + par + 1) * D] for j in range(4)]
                q = pick(cols, r0)
                for b in range(B):
                    g = b * GPB + (k // 2) * 2 + par
                    q_scr[g, r0:r0 + 4, :] = q[b * R + r0:b * R + r0 + 4, :]

        def wo_head(g, r):
            half = (g // 2) % 2
            off = ((2 * r) % 8 + g % 2) * D
            return wo_buf[half * 2 + r // 4, pl.ds(_mult(off, D), D), :]

        def qk(i):
            g = i // PPG
            j = i % G
            q = q_scr[g].astype(_BF16)
            slot = i % NK
            s = pick([_dot_nt(q, kbuf[slot, r]) for r in range(R)])
            s_scr[:, pl.ds(_mult(j * KP, KP), KP)] = s

        def softmax_update():
            s = [s_scr[:, t * 128:(t + 1) * 128] for t in range(KB // 128)]
            mx = functools.reduce(jnp.maximum, s)
            m_old = m_scr[...]
            m_new = jnp.maximum(m_old, jnp.max(mx, axis=1, keepdims=True))
            alpha = jnp.exp((m_old - m_new) * scale)
            p = [jnp.exp((st - m_new) * scale) for st in s]
            l_scr[...] = l_scr[...] * alpha + functools.reduce(jnp.add, p)
            m_scr[...] = m_new
            acc_scr[...] = acc_scr[...] * alpha
            for t in range(KB // 128):
                p_scr[:, t * 128:(t + 1) * 128] = p[t].astype(_BF16)

        def inv_l():
            return 1.0 / jnp.sum(l_scr[...], axis=1, keepdims=True)

        def pv(i):
            j = i % G
            slot = i % NV
            p = p_scr[:, pl.ds(_mult(j * KP, KP), KP)]
            acc_scr[...] += pick([_dot(p, vbuf[slot, r]) for r in range(R)])

        def reset_group():
            acc_scr[...] = jnp.zeros_like(acc_scr)
            l_scr[...] = jnp.zeros_like(l_scr)
            m_scr[...] = jnp.full(m_scr.shape, -jnp.inf, _F32)

        def finish_group(g):
            o = (acc_scr[...] * inv_l()).astype(_BF16)
            oa_scr[g // GPB] += pick([_dot(o, wo_head(g, r)) for r in range(R)])

        def b_init():
            xb16_scr[...] = x16(xb_buf)
            qb_scr[...] = jnp.zeros_like(qb_scr)
            ctxc_scr[...] = jnp.zeros_like(ctxc_scr)

        def b_query(t):
            a, r, tiles = head_tiles(wqb_buf, t)
            x = xb16_scr[:, pl.ds(_mult(r * 128, 128), 128)]
            qb_scr[a] += pick([_dot(x, w) for w in tiles])

        def b_absorb(t):
            a, r, tiles = head_tiles(wuk_buf, t)
            q = qb_scr[a].astype(_BF16)
            qabs = pick([_dot_nt(q, w) for w in tiles])
            for b in range(B):
                qabs_scr[b, pl.ds(_mult(a * 8, 8), 8),
                         pl.ds(_mult(r * 128, 128), 128)] = qabs[b * 8:(b + 1) * 8, :]

        def b_absorb_done():
            qab_scr[...] = qabs_scr[...].astype(_BF16)
            mb_scr[...] = jnp.full(mb_scr.shape, -jnp.inf, _F32)

        NCB = S // CB
        CPR = 1024 // CB

        def ckv_chunk(t):
            b = t // NCB
            j = t % NCB
            return ckv_buf[b * 8 + j // CPR, pl.ds(_mult((j % CPR) * CB, CB), CB), :]

        def b_scores(t):
            b = t // NCB
            j = t % NCB
            s = _dot_nt(qab_scr[b], ckv_chunk(t))
            sb_scr[b, :, pl.ds(_mult(j * CB, CB), CB)] = s
            mb_scr[b] = jnp.maximum(mb_scr[b], fold(s, jnp.maximum))

        def b_scores_done():
            for b in range(B):
                m = jnp.max(mb_scr[b], axis=1, keepdims=True)
                mb_scr[b] = jnp.broadcast_to(m, (H, 128))
            lb_scr[...] = jnp.zeros_like(lb_scr)
            ctx_scr[...] = jnp.zeros_like(ctx_scr)

        def b_ctx(t):
            b = t // NCB
            j = t % NCB
            s = sb_scr[b, :, pl.ds(_mult(j * CB, CB), CB)]
            m = mb_scr[b]
            p = jnp.concatenate(
                [jnp.exp((s[:, u * 128:(u + 1) * 128] - m) * scale)
                 for u in range(CB // 128)], axis=1)
            lb_scr[b] += fold(p, jnp.add)
            ctx_scr[b] += _dot(p.astype(_BF16), ckv_chunk(t))

        def b_ctx_done():
            for b in range(B):
                ctx_scr[b] = ctx_scr[b] / jnp.sum(lb_scr[b], axis=1, keepdims=True)
            ob_scr[...] = jnp.zeros_like(ob_scr)

        def b_value(t):
            a, r, tiles = head_tiles(wuv_buf, t)
            rows = pl.ds(_mult(a * 8, 8), 8)
            cols = pl.ds(_mult(r * 128, 128), 128)
            lhs = jnp.concatenate(
                [ctx_scr[b, rows, cols] for b in range(B)], axis=0).astype(_BF16)
            ctxc_scr[a] += pick([_dot(lhs, w) for w in tiles])

        def b_out(t):
            a = t // 2
            k0 = (t % 2) * 4
            lhs = ctxc_scr[a].astype(_BF16)
            parts = [
                _dot(lhs, wob_buf[a, pl.ds(_mult((k0 + j) * D, D), D), :])
                for j in range(4)
            ]
            k = lax.broadcasted_iota(jnp.int32, (16, M), 0) % 8
            y = jnp.where(k == k0, parts[0], 0.0)
            for j in range(1, 4):
                y = jnp.where(k == k0 + j, parts[j], y)
            ob_scr[...] += y

        def b_done():
            for b in range(B):
                ob = jnp.sum(ob_scr[b * 8:(b + 1) * 8, :], axis=0, keepdims=True)
                out_ref[b:b + 1, M:2 * M] = ob.astype(out_ref.dtype)

        cp_xa.start()
        cp_xb.start()

        def prologue(it, carry):
            for c in range(P):
                ucp(1, 0, it, c).start(priority=_LO)
            return carry

        def prologue_hi(it, carry):
            for c in range(P):
                ucp(0, 0, it, c).start(priority=_HI)
            return carry

        lax.fori_loop(0, XH, prologue_hi, 0)
        lax.fori_loop(0, BV, prologue, 0)

        def first_block(t):
            i = t - (NLO - G)
            kwait_all(i)
            qk(i)

        QA0 = UI + 2

        def plan(t):
            wn, wq_ = lo_seq[t]
            h = hi_seq[t + XH] if t + XH < NHI else (-1, t + XH - NHI)
            l = lo_seq[t + BV] if t + BV < NLO else (-1, t + BV - NLO)
            if QA0 <= t < QA0 + 4:
                ex = ("qa", t - QA0)
            elif t >= NLO - G:
                ex = ("first",)
            else:
                ex = None
            return (wn, h[0], l[0], ex), (wq_ - t, h[1] - t, l[1] - t)

        def phase1_loop(t0, t1):
            (wn, hn, ln, ex), (wo_, ho, lo_) = plan(t0)

            def body(t, carry):
                for c in range(P):
                    ucp(1, wn, t + wo_, c).wait()
                    if hn >= 0:
                        ucp(0, hn, t + ho, c).start(priority=_HI)
                    else:
                        kcp(t + ho, c).start(priority=_HI)
                    if ln >= 0:
                        ucp(1, ln, t + lo_, c).start(priority=_LO)
                    else:
                        vcp(t + lo_, c).start(priority=_LO)
                    if c == 0 and ex is not None:
                        if ex[0] == "qa":
                            qa_task(ex[1])
                        else:
                            first_block(t)
                return carry

            lax.fori_loop(t0, t1, body, 0)

        reset_group()
        oa_scr[...] = jnp.zeros_like(oa_scr)
        t0 = 0
        for t in range(1, NLO + 1):
            if t == NLO or plan(t) != plan(t0):
                if t0 == QA0:
                    hi_run_wait(0)
                    cp_xa.wait()
                    cp_xb.wait()
                phase1_loop(t0, t)
                t0 = t
        for n in range(1, len(hi_runs)):
            hi_run_wait(n)
        softmax_update()
        kwait_all(G)

        def end_of_piece(i):
            @pl.when(i % G == G - 1)
            def _():
                @pl.when(i % PPG == PPG - 1)
                def _():
                    finish_group(i // PPG)
                    reset_group()

                softmax_update()

        def main_loop(lo, hi, extra=None):
            def body(i, carry):
                def issue(c):
                    kcp(i + G + XK, c).start(priority=_HI)
                    vcp(i + BV, c).start(priority=_LO)

                vcp(i, 0).wait()
                issue(0)
                qk(i + G)
                if extra is not None:
                    extra(i - lo)
                for c in range(1, P):
                    vcp(i, c).wait()
                    issue(c)
                pv(i)
                kwait_all(i + G + 1)
                end_of_piece(i)
                return carry

            lax.fori_loop(lo, hi, body, 0)

        def tail_loop(lo, hi):
            def body(i, carry):
                for c in range(P):
                    vcp(i, c).wait()

                    @pl.when(i + BV < NP - G)
                    def _():
                        vcp(i + BV, c).start(priority=_LO)

                    @pl.when(jnp.logical_and(i + BV >= NP - G, i + BV < NP))
                    def _():
                        vcp_last(i + BV, c).start(priority=_LO)

                qk(i + G)
                pv(i)

                @pl.when(i + G + 1 < NP)
                def _():
                    kwait_all(i + G + 1)

                end_of_piece(i)
                return carry

            lax.fori_loop(lo, hi, body, 0)

        def last_block():
            g = NG - 1
            row = lax.broadcasted_iota(jnp.int32, (R, M), 0)
            rl = inv_l()
            y = oa_scr[B - 1]
            for u in range(G):
                i = NP - G + u
                for c in range(P):
                    vcp_last(i, c).wait()
                    if i + BV < NP:
                        vcp_last(i + BV, c).start(priority=_LO)
                slot = i % NV
                rowd = lax.broadcasted_iota(jnp.int32, (R, D), 0)
                o = None
                for e in range(HPP):
                    oe = functools.reduce(jnp.add, [
                        _dot(p_scr[:, kt * KP:(kt + 1) * KP], vbuf[slot, e * G + kt])
                        for kt in range(G)])
                    o = oe if o is None else jnp.where(rowd == u * HPP + e, oe, o)
                o = ((acc_scr[...] + o) * rl).astype(_BF16)
                for e in range(HPP):
                    r = u * HPP + e
                    yr = _dot(o, wo_head(g, r))
                    y = y + jnp.where(row == r, yr, 0.0)
            out_ref[B - 1:B, 0:M] = jnp.sum(y, axis=0, keepdims=True).astype(out_ref.dtype)

        b_init()
        pos = 0
        for n, task, done in [
            (16, b_query, None),
            (16, b_absorb, b_absorb_done),
            (B * NCB, b_scores, b_scores_done),
            (B * NCB, b_ctx, b_ctx_done),
            (16, b_value, None),
            (8, b_out, b_done),
        ]:
            main_loop(pos, pos + n, extra=task)
            pos += n
            if done is not None:
                done()
        tail0 = NP - G - XK
        assert XK >= BV - G
        assert pos <= tail0 and P % G == 0 and HPP * G == R and P == R
        main_loop(pos, tail0)
        for b in range(B - 1):
            oa = jnp.sum(oa_scr[b], axis=0, keepdims=True)
            out_ref[b:b + 1, 0:M] = oa.astype(out_ref.dtype)
        tail_loop(tail0, NP - G)
        last_block()

    scratch = [
        pltpu.VMEM((B, M), _BF16),
        pltpu.VMEM((B, M), _BF16),
        pltpu.VMEM((8, 64, HD), _BF16),
        pltpu.VMEM((4, 1024, M), _BF16),
        pltpu.VMEM((4, 4096, D), _BF16),
        pltpu.VMEM((4, 4096, D), _BF16),
        pltpu.VMEM((4, 4096, D), _BF16),
        pltpu.VMEM((4, 1024, M), _BF16),
        pltpu.VMEM((16, 1024, M), _BF16),
        pltpu.VMEM((NK, R, KP, D), _BF16),
        pltpu.VMEM((NV, R, KP, D), _BF16),
        pltpu.VMEM((NG, R, D), _F32),
        pltpu.VMEM((R, KB), _F32),
        pltpu.VMEM((R, KB), _BF16),
        pltpu.VMEM((R, D), _F32),
        pltpu.VMEM((R, D), _F32),
        pltpu.VMEM((R, D), _F32),
        pltpu.VMEM((B, R, M), _F32),
        pltpu.VMEM((16, M), _BF16),
        pltpu.VMEM((GPB, 16, D), _F32),
        pltpu.VMEM((B, H, M), _F32),
        pltpu.VMEM((B, H, M), _BF16),
        pltpu.VMEM((B, H, S), _F32),
        pltpu.VMEM((B, H, 128), _F32),
        pltpu.VMEM((B, H, 128), _F32),
        pltpu.VMEM((B, H, M), _F32),
        pltpu.VMEM((GPB, 16, D), _F32),
        pltpu.VMEM((16, M), _F32),
    ]

    def call(A_x, A_k_cache, A_v_cache, A_wq, A_wo, B_x, B_c_kv, B_w_q, B_w_uk,
             B_w_uv, B_w_o):
        any_spec = pl.BlockSpec(memory_space=pl.ANY)
        out = pl.pallas_call(
            kernel,
            out_shape=jax.ShapeDtypeStruct((B, 2 * M), _BF16),
            in_specs=[any_spec] * 11,
            out_specs=pl.BlockSpec(memory_space=pltpu.VMEM),
            scratch_shapes=scratch,
            compiler_params=pltpu.CompilerParams(
                vmem_limit_bytes=100 * 1024 * 1024,
                disable_bounds_checks=True),
        )(
            A_x.reshape(B, M),
            A_k_cache.reshape(B * 2, R, 2, S, D),
            A_v_cache.reshape(B * 2, R, 2, S, D),
            A_wq.reshape(8, 64, HD),
            A_wo.reshape(4, 1024, M),
            B_x.reshape(B, M),
            B_c_kv.reshape(16, 1024, M),
            B_w_q.reshape(4, 4096, D),
            B_w_uk.reshape(4, 4096, D),
            B_w_uv.reshape(4, 4096, D),
            B_w_o.reshape(4, 1024, M),
        )
        return out.reshape(B, 1, 2 * M)

    return call


@jax.jit
def pallas_concat_heads__gqa_block_cached__compressed_kv_cla__decode_kernel(
    A_x: jax.Array,
    A_k_cache: jax.Array,
    A_v_cache: jax.Array,
    A_wq: jax.Array,
    A_wo: jax.Array,
    B_x: jax.Array,
    B_c_kv: jax.Array,
    B_w_q: jax.Array,
    B_w_uk: jax.Array,
    B_w_uv: jax.Array,
    B_w_o: jax.Array,
):
    B, H, S, D = A_k_cache.shape
    M = A_x.shape[-1]
    assert A_x.shape == (B, 1, M) and B_x.shape == (B, 1, M)
    assert A_wq.shape == (M, H * D) and B_c_kv.shape == (B, S, M)
    assert B_w_q.shape == (M, H, D) and B_w_o.shape == (H, D, M)
    return _build(B, H, S, D, M)(A_x, A_k_cache, A_v_cache, A_wq, A_wo, B_x,
                                 B_c_kv, B_w_q, B_w_uk, B_w_uv, B_w_o)
```
